```python
import jax
import jax.numpy as jnp

def _softmax(x, axis=-1):
    return jax.nn.softmax(x, axis=axis)
def _gelu(x):
    return jax.nn.gelu(x, approximate=True)
def _silu(x):
    return jax.nn.silu(x)
def _sigmoid(x):
    return jax.nn.sigmoid(x)
def _layernorm(x, axis=-1, eps=1e-5):
    m = jnp.mean(x, axis=axis, keepdims=True)
    v = jnp.var(x, axis=axis, keepdims=True)
    return (x - m) / jnp.sqrt(v + eps)
def _scatter_add(tgt, idx, src, axis=0):
    return tgt.at[idx].add(src)
def _segment_sum(src, seg, n):
    return jax.ops.segment_sum(src, seg, n)
class _Rng:
    def __init__(self, key):
        self._k = key
    def _next(self):
        self._k, sub = jax.random.split(self._k)
        return sub
    def normal(self, shape):
        return jax.random.normal(self._next(), shape, dtype=jnp.bfloat16)
    def randint(self, lo, hi, shape):
        return jax.random.randint(self._next(), shape, lo, hi, dtype=jnp.int32)
    def uniform(self, shape, lo=0.0, hi=1.0):
        return jax.random.uniform(self._next(), shape, jnp.bfloat16, lo, hi)
    def permutation(self, n):
        return jax.random.permutation(self._next(), n)


kernel_name = 'standalone__batchnorm__prompt'

def setup_inputs():
    _rng = _Rng(jax.random.key(int.from_bytes(__import__("os").urandom(4), "little")))
    _w = (lambda a: (lambda t: t.astype(jnp.bfloat16) if jnp.issubdtype(t.dtype, jnp.floating) else t)(jnp.asarray(a)))
    B, S, C = 2, 2048, 1024
    K = 3
    return {
        "x": _w((lambda *s: _rng.normal(s) * 0.05)(B, S, C)),
        "w": _w((lambda *s: _rng.normal(s) * 0.05)(K, C, C) * (1.0 / (K * C) ** 0.5)),
        "mean": _w((lambda *s: _rng.normal(s) * 0.05)(C) * 0.1),
        "var": _w(jnp.abs((lambda *s: _rng.normal(s) * 0.05)(C)) + 0.5),
        "g": _w((lambda *s: _rng.normal(s) * 0.05)(C) + 1.0),
        "b": _w((lambda *s: _rng.normal(s) * 0.05)(C) * 0.1),
    }

def reference(x, w, mean, var, g, b):
    K = 3
    P = K // 2
    S = x.shape[1]
    xp = jnp.pad(x, ((0, 0), (P, P), (0, 0)))
    y = sum(jnp.einsum('bsc,cd->bsd', xp[:, k:k + S, :], w[k]) for k in range(K))
    inv_std = 1.0 / jnp.sqrt(var + 1e-5)
    y = (y - mean) * (g * inv_std) + b
    return _silu(y)
```

```python
import functools
import jax, jax.numpy as jnp
import jax.experimental.pallas as pl
import jax.experimental.pallas.tpu as pltpu

A = 2.0/3.0; Bp = 1.5
A2 = A*A; B2 = Bp*Bp; PP = A2 + B2
NA = 2*A2*(A2-B2); NB = 2*B2*(B2-A2)
f32 = jnp.float32; bf16 = jnp.bfloat16; i32 = jnp.int32

def lo(wd): return pltpu.unpack_elementwise(wd, index=0, packed_dtype=bf16, unpacked_dtype=f32)
def hi(wd): return pltpu.unpack_elementwise(wd, index=1, packed_dtype=bf16, unpacked_dtype=f32)
def pk(a, b): return pltpu.pack_elementwise((a, b), packed_dtype=bf16)

def silu(z, mode):
    if mode == 0:
        return z * jax.nn.sigmoid(z)
    h = 0.5 * z
    return h + h * jnp.tanh(h)

def kern(x_ref, w_ref, mean_ref, var_ref, g_ref, b_ref, o_ref, gw_ref, *, T, S, mode):
    bi = pl.program_id(0); i = pl.program_id(1)
    C = x_ref.shape[-1]
    R = 4*T
    @pl.when((bi == 0) & (i == 0))
    def _():
        def body(j, c):
            r = pl.ds(pl.multiple_of(j*128, 128), 128)
            w0 = w_ref[0, r, :].astype(f32); w1 = w_ref[1, r, :].astype(f32); w2 = w_ref[2, r, :].astype(f32)
            sa = w0*(1.0/NA) + w2*(A2/NA); da = w1*(A/NA)
            sb = w0*(1.0/NB) + w2*(B2/NB); db = w1*(Bp/NB)
            gw_ref[0, r, :] = (sa + da).astype(bf16)
            gw_ref[1, r, :] = (sa - da).astype(bf16)
            gw_ref[2, r, :] = (sb + db).astype(bf16)
            gw_ref[3, r, :] = (sb - db).astype(bf16)
            return c
        jax.lax.fori_loop(0, C//128, body, 0)
    ld = lambda r: r[...].astype(f32).reshape(1, C)
    mean = ld(mean_ref); var = ld(var_ref); g = ld(g_ref); b = ld(b_ref)
    scale = g * jax.lax.rsqrt(var + 1e-5)
    shift = b - mean*scale
    s0 = pl.multiple_of(i*R, R)
    lo_s = jnp.maximum(s0-32, 0); hi_s = jnp.minimum(s0+R, S-32)
    def deint(xw):
        E = lo(xw); O = hi(xw)
        Ew = pltpu.bitcast(E.astype(bf16), i32); Ow = pltpu.bitcast(O.astype(bf16), i32)
        return lo(Ew), lo(Ow), hi(Ew), hi(Ow)
    xc = pltpu.bitcast(x_ref[pl.ds(s0, R), :], i32)
    xl = pltpu.bitcast(x_ref[pl.ds(pl.multiple_of(lo_s,32), 32), :], i32)
    xh = pltpu.bitcast(x_ref[pl.ds(pl.multiple_of(hi_s,32), 32), :], i32)
    xl = jnp.where(i > 0, xl, 0); xh = jnp.where(i < S//R-1, xh, 0)
    d1, d2, d3, d4 = deint(xc)
    d4l = deint(xl)[3]; d1h = deint(xh)[0]
    d0 = pltpu.roll(jnp.concatenate([d4l, d4], axis=0), 1, 0)[8:]
    d5 = pltpu.roll(jnp.concatenate([d1, d1h], axis=0), T+8-1, 0)[:T]
    t0 = ((d0 + d4) - PP*d2).astype(bf16)
    t5 = ((d1 + d5) - PP*d3).astype(bf16)
    u1 = d4 - B2*d2; v1 = A*(d3 - B2*d1)
    u2 = d4 - A2*d2; v2 = Bp*(d3 - A2*d1)
    t1 = (u1+v1).astype(bf16); t2 = (u1-v1).astype(bf16)
    t3 = (u2+v2).astype(bf16); t4 = (u2-v2).astype(bf16)
    dot = lambda a, bb: jnp.dot(a, bb, preferred_element_type=f32)
    m0 = dot(t0, w_ref[0]); m5 = dot(t5, w_ref[2])
    m1 = dot(t1, gw_ref[0]); m2 = dot(t2, gw_ref[1])
    m3 = dot(t3, gw_ref[2]); m4 = dot(t4, gw_ref[3])
    sa = m1 + m2; da = m1 - m2; sb = m3 + m4; db = m3 - m4
    y0 = m0 + sa + sb
    y1 = A*da + Bp*db
    y2 = A2*sa + B2*sb
    y3 = (A*A2)*da + (Bp*B2)*db + m5
    y0, y1, y2, y3 = [silu(y*scale + shift, mode) for y in (y0, y1, y2, y3)]
    Ew = pk(y0, y2); Ow = pk(y1, y3)
    Ef = pltpu.bitcast(Ew, bf16).astype(f32); Of = pltpu.bitcast(Ow, bf16).astype(f32)
    o_ref[...] = pltpu.bitcast(pk(Ef, Of), bf16)

@jax.jit
def pallas_standalone__batchnorm__prompt_kernel(x, w, mean, var, g, b):
    return run(x, w, mean, var, g, b)

def run(x, w, mean, var, g, b, T=128, mode=1):
    B,S,C = x.shape
    r2 = lambda a: a
    vec = pl.BlockSpec((C,), lambda bi,i: (0,))
    return pl.pallas_call(
        functools.partial(kern, T=T, S=S, mode=mode),
        grid=(B, S//(4*T)),
        in_specs=[pl.BlockSpec((None,S,C), lambda bi,i:(bi,0,0)),
                  pl.BlockSpec((3,C,C), lambda bi,i:(0,0,0), pipeline_mode=pl.Buffered(1)),
                  vec,vec,vec,vec],
        out_specs=pl.BlockSpec((None,4*T,C), lambda bi,i:(bi,i,0)),
        out_shape=jax.ShapeDtypeStruct((B,S,C), x.dtype),
        scratch_shapes=[pltpu.VMEM((4,C,C), bf16)],
        compiler_params=pltpu.CompilerParams(dimension_semantics=("arbitrary","arbitrary"), vmem_limit_bytes=100*1024*1024),
    )(x, w, r2(mean), r2(var), r2(g), r2(b))
```

```python
import functools
import jax, jax.numpy as jnp
import jax.experimental.pallas as pl
import jax.experimental.pallas.tpu as pltpu

A = 2.0/3.0; Bp = 1.5
A2 = A*A; B2 = Bp*Bp; PP = A2 + B2
NA = 2*A2*(A2-B2); NB = 2*B2*(B2-A2)
f32 = jnp.float32; bf16 = jnp.bfloat16; i32 = jnp.int32

def lo(wd): return pltpu.unpack_elementwise(wd, index=0, packed_dtype=bf16, unpacked_dtype=f32)
def hi(wd): return pltpu.unpack_elementwise(wd, index=1, packed_dtype=bf16, unpacked_dtype=f32)
def pk(a, b): return pltpu.pack_elementwise((a, b), packed_dtype=bf16)

def kern(x_hbm, w_hbm, mean_ref, var_ref, g_ref, b_ref, o_hbm,
         xbuf, wbuf, gbuf, tb, obuf, xsem, wsem, osem, zsem, *, T, Nc, XG, XC, EG, GR, GC, xdots, gdots, xsplit, anchor, x1units, aoff, porder):
    B, S, C = x_hbm.shape
    R = 4*T
    tiles = [(b, i) for b in range(B) for i in range(S//R)]
    NT = len(tiles); NCH = C//Nc
    per = S//R

    def x_copy(ti, p=0, np_=1):
        b, i = tiles[ti]
        r0 = R*i + (16 if i > 0 else 0)
        r1 = R*(i+1) + (16 if i < per-1 else 0)
        if np_ > 1:
            q0 = R*i + p*R//np_ + 16; q1 = R*i + (p+1)*R//np_ + 16
            r0 = r0 if p == 0 else q0
            r1 = r1 if p == np_-1 else q1
        return pltpu.make_async_copy(x_hbm.at[b, pl.ds(r0, r1-r0), :], xbuf.at[b, pl.ds(r0, r1-r0), :], xsem.at[ti, p])
    def w_copy(c, k):
        cols = pl.ds(c*Nc, Nc)
        return pltpu.make_async_copy(w_hbm.at[k, :, cols], wbuf.at[k, :, cols], wsem.at[c, k])
    def o_copy(ti, c):
        b, i = tiles[ti]
        cols = pl.ds(c*Nc, Nc); rows = pl.ds(R*i, R)
        return pltpu.make_async_copy(obuf.at[b, rows, cols], o_hbm.at[b, rows, cols], osem.at[ti, c])

    ld = lambda r: r[...].astype(f32).reshape(1, C)
    mean = ld(mean_ref); var = ld(var_ref); g = ld(g_ref); bb = ld(b_ref)
    scale = 0.5 * g * jax.lax.rsqrt(var + 1e-5)
    shift = 0.5 * bb - mean*scale
    zvec = jnp.full((8, 128), pl.semaphore_read(zsem), i32)

    def dep_of(m, rb):
        return pltpu.bitcast(m[rb*8:(rb+1)*8, 0:128], i32) & zvec
    def tile_dep(dep, rows, cols):
        return jnp.concatenate([jnp.concatenate([dep]*(cols//128), axis=1)]*(rows//8), axis=0)

    def xload(ti, gp, cp):
        b, i = tiles[ti]
        ng = XG
        row0 = R*i + 4*gp*ng
        cols = pl.ds(cp*XC, XC)
        xc = pltpu.bitcast(xbuf[b, pl.ds(row0, 4*ng), cols], i32)
        pw = pltpu.bitcast(xbuf[b, pl.ds(row0-16, 16), cols], i32) if row0 > 0 else None
        nw = pltpu.bitcast(xbuf[b, pl.ds(row0+4*ng, 16), cols], i32) if row0 + 4*ng < S else None
        return xc, pw, nw

    def xtr(ti, gp, cp, dep=None, loaded=None):
        b, i = tiles[ti]
        ng = XG
        g0 = gp*ng
        row0 = R*i + 4*g0
        cols = pl.ds(cp*XC, XC)
        xc, pw, nw = loaded if loaded is not None else xload(ti, gp, cp)
        if dep is not None: xc = xc | tile_dep(dep, 2*ng, XC)
        E = lo(xc); O = hi(xc)
        Ew = pltpu.bitcast(E.astype(bf16), i32); Ow = pltpu.bitcast(O.astype(bf16), i32)
        d1, d2, d3, d4 = lo(Ew), lo(Ow), hi(Ew), hi(Ow)
        if row0 > 0:
            if dep is not None and anchor > 1: pw = pw | tile_dep(dep, 8, XC)
            prev = hi(pw)
        else:
            prev = jnp.zeros((8, XC), f32)
        if row0 + 4*ng < S:
            if dep is not None and anchor > 1: nw = nw | tile_dep(dep, 8, XC)
            nxt = lo(nw)
        else:
            nxt = jnp.zeros((8, XC), f32)
        d0 = pltpu.roll(jnp.concatenate([prev, d4], axis=0), 1, 0)[8:]
        d5 = pltpu.roll(jnp.concatenate([d1, nxt], axis=0), ng+8-1, 0)[:ng]
        rows = pl.ds((ti*T + g0)//2, ng//2)
        def st(j, v): tb[j, rows, cols] = pltpu.bitcast(v.astype(bf16), i32)
        st(0, (d0 + d4) - PP*d2)
        st(5, (d1 + d5) - PP*d3)
        u1 = d4 - B2*d2; v1 = A*(d3 - B2*d1)
        st(1, u1+v1); st(2, u1-v1)
        u2 = d4 - A2*d2; v2 = Bp*(d3 - A2*d1)
        st(3, u2+v2); st(4, u2-v2)

    def gload(c, rp, cp):
        cols = pl.ds(c*Nc + cp*GC, GC)
        rows = pl.ds(rp*GR, GR)
        return [pltpu.bitcast(wbuf[k, rows, cols], i32) for k in range(3)]

    def orall(vals):
        acc = None
        for v in vals:
            if v is None: continue
            for r in range(v.shape[0]//8):
                for q in range(v.shape[1]//128):
                    t = v[8*r:8*r+8, 128*q:128*q+128]
                    acc = t if acc is None else acc | t
        return acc

    def gtr(c, rp, cp, dep=None, loaded=None):
        cols = pl.ds(c*Nc + cp*GC, GC)
        rows = pl.ds(rp*GR, GR); hrows = pl.ds(rp*GR//2, GR//2)
        wv = loaded if loaded is not None else gload(c, rp, cp)
        if dep is not None:
            dd = tile_dep(dep, GR//2, GC)
            wv = [v | dd for v in wv]
        gbuf[0, hrows, cols] = wv[0]; gbuf[5, hrows, cols] = wv[2]
        res = []
        for h in (lo, hi):
            w0, w1, w2 = h(wv[0]), h(wv[1]), h(wv[2])
            sa = w0*(1.0/NA) + w2*(A2/NA); da = w1*(A/NA)
            sb = w0*(1.0/NB) + w2*(B2/NB); db = w1*(Bp/NB)
            res.append((sa+da, sa-da, sb+db, sb-db))
        for j in range(4):
            gbuf[1+j, hrows, cols] = pk(res[0][j], res[1][j])

    def epi(ti, c, ms, part):
        b, i = tiles[ti]
        ng = EG
        sl = slice(part*ng, (part+1)*ng)
        m0, m1, m2, m3, m4, m5 = [m[sl] for m in ms]
        sa = m1 + m2; da = m1 - m2; sb = m3 + m4; db = m3 - m4
        y0 = m0 + sa + sb
        y1 = A*da + Bp*db
        y2 = A2*sa + B2*sb
        y3 = (A*A2)*da + (Bp*B2)*db + m5
        sc = scale[:, c*Nc:(c+1)*Nc]; sh = shift[:, c*Nc:(c+1)*Nc]
        def act(y):
            h = y*sc + sh
            return h + h*jnp.tanh(h)
        y0, y1, y2, y3 = act(y0), act(y1), act(y2), act(y3)
        Ef = pltpu.bitcast(pk(y0, y2), bf16).astype(f32); Of = pltpu.bitcast(pk(y1, y3), bf16).astype(f32)
        obuf[b, pl.ds(R*i + 4*part*ng, 4*ng), pl.ds(c*Nc, Nc)] = pltpu.bitcast(pk(Ef, Of), bf16)

    xargs = [(gp, cp) for gp in range(T//XG) for cp in range(C//XC)]
    gargs = [(rp, cp) for rp in range(C//GR) for cp in range(Nc//GC)]
    WK = (0, 2, 1)

    for k in WK: w_copy(0, k).start()
    x_copy(0, 0, xsplit).start()
    for k in WK: w_copy(0, k).wait()
    if xsplit > 1: x_copy(0, 1, xsplit).start()
    for a in gargs: gtr(0, *a)
    n = len(xargs)
    for p in range(xsplit):
        x_copy(0, p, xsplit).wait()
        if p+2 < xsplit: x_copy(0, p+2, xsplit).start()
        if p+2 == xsplit or xsplit == 1:
            for k in WK: w_copy(1, k).start()
        for a in xargs[p*n//xsplit:(p+1)*n//xsplit]: xtr(0, *a)

    started = {('w', 0), ('w', 1), ('x', 0)}
    def wwait(c):
        assert ('w', c) in started
        for k in WK: w_copy(c, k).wait()
    def xwait(t):
        assert ('x', t) in started
        x_copy(t).wait()
    def kick(kind, n):
        assert (kind, n) not in started
        started.add((kind, n))
        if kind == 'w':
            for k in WK: w_copy(n, k).start()
        else:
            x_copy(n).start()
    starts = {(0, 2): [('w', 2)], (1, 0): [('w', 3)], (1, 4): [('x', 1)], (2, 4): [('x', 2)], (3, 4): [('x', 3)]}
    units = [(ti, c) for ti in range(NT) for c in range(NCH)]
    RB = T//8
    for u, (ti, c) in enumerate(units):
        rows = pl.ds(ti*T//2, T//2)
        xs = []
        if ti+1 < NT:
            if ti == 0:
                us = list(range(NCH - x1units, NCH))
                if c in us:
                    k_ = us.index(c); xs = xargs[k_*n//len(us):(k_+1)*n//len(us)]
            else:
                xs = xargs[c*n//NCH:(c+1)*n//NCH]
        gs = gargs if (ti == 0 and c+1 < NCH) else []
        ms = []
        for j in range(6):
            mine = []
            if xs and j in xdots:
                k_ = xdots.index(j); mx = xs[k_*len(xs)//len(xdots):(k_+1)*len(xs)//len(xdots)]
                if k_ == 0:
                    first = (ti == 0 and c == NCH - x1units) or (ti > 0 and c == 0)
                    if first:
                        xwait(ti+1)
                mine += [(xtr, (ti+1,)+a) for a in mx]
            if gs and j in gdots:
                k_ = gdots.index(j); mg = gs[k_*len(gs)//len(gdots):(k_+1)*len(gs)//len(gdots)]
                if k_ == 0:
                    wwait(c+1)
                mine += [(gtr, (c+1,)+a) for a in mg]
            for kd in starts.get((u, j), []): kick(*kd)
            lhs = pltpu.bitcast(tb[j, rows, :], bf16)
            rw = gbuf[j, :, pl.ds(c*Nc, Nc)]
            loaded = []
            if anchor == 3 and mine:
                NTL = Nc//128
                NP = NTL*2*32
                mod = {}
                for q, (fn, a) in enumerate(mine):
                    ldv = (xload if fn is xtr else gload)(*a)
                    loaded.append(ldv)
                    p = ((2*q+1)*NP)//(2*len(mine))
                    p = min(NP-1, max(0, p - aoff))
                    ps, r_ = p//32, p % 32
                    if porder == 0: nt, kg = ps//2, ps % 2
                    else: nt, kg = ps % NTL, ps//NTL
                    kt = 4*kg + (r_ % 4); sb = r_//4
                    mod[(kt*8 + sb, nt)] = orall(ldv) & zvec
                rowsb = []
                for rbk in range(C//16):
                    blk = rw[8*rbk:8*rbk+8]
                    if any(k_[0] == rbk for k_ in mod):
                        blk = jnp.concatenate([(blk[:, 128*nt:128*nt+128] | mod[(rbk, nt)]) if (rbk, nt) in mod else blk[:, 128*nt:128*nt+128] for nt in range(NTL)], axis=1)
                    rowsb.append(blk)
                rw = jnp.concatenate(rowsb, axis=0)
            rhs = pltpu.bitcast(rw, bf16)
            m = jnp.dot(lhs, rhs, preferred_element_type=f32)
            ms.append(m)
            for q, (fn, a) in enumerate(mine):
                rb = (q*RB)//len(mine)
                if anchor == 3: fn(*a, loaded=loaded[q])
                else: fn(*a, dep=dep_of(m, rb) if anchor else None)
        for p in range(T//EG): epi(ti, c, ms, p)
        o_copy(ti, c).start()
    for ti, c in units: o_copy(ti, c).wait()

def _run(x, w, mean, var, g, b, T=256, Nc=256, XG=16, XC=256, EG=16, GR=16, GC=256, xdots=13, gdots=345, xsplit=4, anchor=1, x1units=1, aoff=0, porder=0):
    B,S,C = x.shape
    NT = B*S//(4*T); NCH = C//Nc
    assert NCH == 4 and NT == 4
    xdots = [int(ch) for ch in str(xdots).zfill(2)] if not isinstance(xdots, str) else [int(ch) for ch in xdots[1:]]
    gdots = [int(ch) for ch in str(gdots)] if not isinstance(gdots, str) else [int(ch) for ch in gdots[1:]]
    vec = pl.BlockSpec(memory_space=pltpu.VMEM)
    hbm = pl.BlockSpec(memory_space=pl.ANY)
    return pl.pallas_call(
        functools.partial(kern, T=T, Nc=Nc, XG=XG, XC=XC, EG=EG, GR=GR, GC=GC, xdots=xdots, gdots=gdots, xsplit=xsplit, anchor=anchor, x1units=x1units, aoff=aoff, porder=porder),
        in_specs=[hbm, hbm, vec, vec, vec, vec],
        out_specs=hbm,
        out_shape=jax.ShapeDtypeStruct((B,S,C), x.dtype),
        scratch_shapes=[
            pltpu.VMEM((B,S,C), bf16), pltpu.VMEM((3,C,C), bf16), pltpu.VMEM((6,C//2,C), i32),
            pltpu.VMEM((6,B*S//8,C), i32), pltpu.VMEM((B,S,C), bf16),
            pltpu.SemaphoreType.DMA((NT,8)), pltpu.SemaphoreType.DMA((NCH,3)), pltpu.SemaphoreType.DMA((NT,NCH)),
            pltpu.SemaphoreType.REGULAR,
        ],
        compiler_params=pltpu.CompilerParams(vmem_limit_bytes=100*1024*1024),
    )(x, w, mean, var, g, b)


@jax.jit
def pallas_standalone__batchnorm__prompt_kernel(x, w, mean, var, g, b):
    return _run(x, w, mean, var, g, b, xdots='s01234', anchor=3, XC=128, GC=128, gdots='s2345')
```

```python
import functools
import jax, jax.numpy as jnp
import jax.experimental.pallas as pl
import jax.experimental.pallas.tpu as pltpu

A = 2.0/3.0; Bp = 1.5
A2 = A*A; B2 = Bp*Bp; PP = A2 + B2
NA = 2*A2*(A2-B2); NB = 2*B2*(B2-A2)
f32 = jnp.float32; bf16 = jnp.bfloat16; i32 = jnp.int32

def lo(wd): return pltpu.unpack_elementwise(wd, index=0, packed_dtype=bf16, unpacked_dtype=f32)
def hi(wd): return pltpu.unpack_elementwise(wd, index=1, packed_dtype=bf16, unpacked_dtype=f32)
def pk(a, b): return pltpu.pack_elementwise((a, b), packed_dtype=bf16)

def kern(x_hbm, w_hbm, mean_hbm, var_hbm, g_hbm, b_hbm, o_hbm,
         xbuf, wbuf, gbuf, tb, obuf, vb0, vb1, vb2, vb3, xsem, wsem, osem, vsem, zsem, *,
         T, NC0, NC1, XG, GR, xdepth, wp0, wp1, xdots, gdots, xsplit, x1units, wk, xk, osplit, nunits, jorder, odefer, orate, x2skip):
    B, S, C = x_hbm.shape
    R = 4*T
    tiles = [(b, i) for b in range(B) for i in range(S//R)]
    NT = len(tiles)
    per = S//R
    NQ = C//128
    EG = 16
    PAD = 16
    xi = xbuf.bitcast(i32); wi = wbuf.bitcast(i32); oi = obuf.bitcast(i32)

    def x_copies(ti, p=0, np_=1):
        b, i = tiles[ti]
        r0 = R*i + (16 if i > 0 else 0)
        r1 = R*(i+1) + (16 if i < per-1 else 0)
        if np_ > 1:
            r0 = r0 if p == 0 else R*i + p*R//np_ + 16
            r1 = r1 if p == np_-1 else R*i + (p+1)*R//np_ + 16
        return [pltpu.make_async_copy(x_hbm.at[b, pl.ds(r0, r1-r0), pl.ds(ct*128, 128)], xbuf.at[b, ct, pl.ds(PAD + r0, r1-r0), :], xsem.at[ti, p])
                for ct in range(NQ)]
    def w_copies(q):
        return [pltpu.make_async_copy(w_hbm.at[:, :, pl.ds(q*128, 128)], wbuf.at[:, q], wsem.at[q])]
    v_copies = [pltpu.make_async_copy(r, d_, vsem.at[n]) for n, (r, d_) in enumerate(zip((mean_hbm, var_hbm, g_hbm, b_hbm), (vb0, vb1, vb2, vb3)))]

    zvec = jnp.full((8, 128), pl.semaphore_read(zsem), i32)

    def xload(ti, gp, cp):
        b, i = tiles[ti]
        out = []
        for h in range(2):
            base = (PAD + R*i)//2 + 2*(gp*XG + 8*h)
            out += [xi[b, cp, pl.ds(base + o, 8, stride=2), :] for o in (-1, 0, 1, 2)]
        return out

    def xtr(ti, gp, cp, loaded=None):
        ld_ = loaded if loaded is not None else xload(ti, gp, cp)
        ts = []
        for h in range(2):
            wa, wb, wc, wd = ld_[4*h:4*h+4]
            d0, d1, d2, d3, d4, d5 = hi(wa), lo(wb), hi(wb), lo(wc), hi(wc), lo(wd)
            u1 = d4 - B2*d2; v1 = A*(d3 - B2*d1)
            u2 = d4 - A2*d2; v2 = Bp*(d3 - A2*d1)
            ts.append(((d0 + d4) - PP*d2, u1+v1, u1-v1, u2+v2, u2-v2, (d1 + d5) - PP*d3))
        rows = pl.ds((ti*T + gp*XG)//2, 8)
        for j in range(6):
            tb[j, rows, pl.ds(cp*128, 128)] = pk(ts[0][j], ts[1][j])

    def gload(q, rp):
        return [wi[k, q, pl.ds(rp*GR//2, GR//2), :] for k in range(3)]
    def gtr(q, rp, loaded=None):
        wv = loaded if loaded is not None else gload(q, rp)
        res = []
        for h in (lo, hi):
            w0, w1, w2 = h(wv[0]), h(wv[1]), h(wv[2])
            sa = w0*(1.0/NA) + w2*(A2/NA); da = w1*(A/NA)
            sb = w0*(1.0/NB) + w2*(B2/NB); db = w1*(Bp/NB)
            res.append((sa+da, sa-da, sb+db, sb-db))
        for j in range(4):
            gbuf[j, pl.ds(rp*GR//2, GR//2), pl.ds(q*128, 128)] = pk(res[0][j], res[1][j])

    def orall(vals):
        acc = None
        for v in vals:
            if v is None: continue
            for r in range(v.shape[0]//8):
                for q in range(v.shape[1]//128):
                    t = v[8*r:8*r+8, 128*q:128*q+128]
                    acc = t if acc is None else acc | t
        return acc

    for p in range(min(xdepth, xsplit)):
        for cp_ in x_copies(0, p, xsplit): cp_.start()
    for cp_ in v_copies: cp_.start()
    zpad = jnp.zeros((PAD//2, 128), i32)
    for b_ in range(B):
        for ct in range(NQ):
            xi[b_, ct, pl.ds(0, PAD//2), :] = zpad
            xi[b_, ct, pl.ds((PAD + S)//2, PAD//2), :] = zpad
    xargs = [(gp, cp) for gp in range(T//XG) for cp in range(NQ)]
    gargs = list(range(C//GR))
    n = len(xargs)
    started = set()
    def kick(kind, m):
        assert (kind, m) not in started
        started.add((kind, m))
        if kind == 'w':
            for cp_ in w_copies(m): cp_.start()
        else:
            for cp_ in x_copies(m): cp_.start()
    for p in range(xsplit):
        for cp_ in x_copies(0, p, xsplit): cp_.wait()
        if p+xdepth < xsplit:
            for cp_ in x_copies(0, p+xdepth, xsplit): cp_.start()
        if p == min(xsplit-1, wp0): kick('w', 0)
        if p == min(xsplit-1, wp1): kick('w', 1)
        for a in xargs[p*n//xsplit:(p+1)*n//xsplit]: xtr(0, *a)
    for cp_ in v_copies: cp_.wait()
    mean, var, g, bb = [r[...].astype(f32).reshape(1, C) for r in (vb0, vb1, vb2, vb3)]
    scale = 0.5 * g * jax.lax.rsqrt(var + 1e-5)
    shift = 0.5 * bb - mean*scale

    def epi(ti, c0, nc, ms, part):
        b, i = tiles[ti]
        sl = slice(part*EG, (part+1)*EG)
        m0, m1, m2, m3, m4, m5 = [ms[j][sl] for j in range(6)]
        sa = m1 + m2; da = m1 - m2; sb = m3 + m4; db = m3 - m4
        y0 = m0 + sa + sb
        y1 = A*da + Bp*db
        y2 = A2*sa + B2*sb
        y3 = (A*A2)*da + (Bp*B2)*db + m5
        sc = scale[:, c0:c0+nc]; sh = shift[:, c0:c0+nc]
        def act(y):
            h = y*sc + sh
            return h + h*jnp.tanh(h)
        y0, y1, y2, y3 = act(y0), act(y1), act(y2), act(y3)
        W01 = pk(y0, y1); W23 = pk(y2, y3)
        ev = jax.lax.broadcasted_iota(i32, (8, nc), 0) % 2 == 0
        wbase = (R*i + 4*part*EG)//2
        for h in range(2):
            a_ = W01[8*h:8*h+8]; b_ = W23[8*h:8*h+8]
            t_lo = jnp.where(ev, a_, pltpu.roll(b_, 1, 0))
            t_hi = jnp.where(ev, pltpu.roll(a_, 7, 0), b_)
            for q in range(nc//128):
                ct = c0//128 + q
                oi[b, ct, pl.ds(wbase + 8*h, 8), :] = t_lo[:, 128*q:128*q+128]
                oi[b, ct, pl.ds(wbase + 16 + 8*h, 8), :] = t_hi[:, 128*q:128*q+128]

    units = [(0, c0, NC0) for c0 in range(0, C, NC0)] + [(ti, c0, NC1) for ti in range(1, NT) for c0 in range(0, C, NC1)]
    units = units[:nunits]
    waited = set()
    def wait(kind, m):
        assert (kind, m) in started, (kind, m)
        if (kind, m) in waited: return
        waited.add((kind, m))
        if kind == 'w':
            for cp_ in w_copies(m): cp_.wait()
        else:
            for cp_ in x_copies(m): cp_.wait()
    starts = {}
    for q in range(2, NQ): starts.setdefault(wk[0] + ((q-2)*wk[1])//10, []).append(('w', q))
    for t in range(1, NT): starts.setdefault(xk[t-1], []).append(('x', t))
    pending_out = []
    def flush_out(k_):
        for _ in range(min(k_, len(pending_out))): pending_out.pop(0).start()
    o_copies = []
    RB = T//8
    gdot = 0
    nu0 = C//NC0
    for u, (ti, c0, nc) in enumerate(units):
        rows = pl.ds(ti*T//2, T//2)
        ntl = nc//128
        xs = []
        if ti+1 < NT:
            if ti == 0:
                us = list(range(nu0 - x1units, nu0))
                if u in us:
                    k_ = us.index(u); xs = xargs[k_*n//len(us):(k_+1)*n//len(us)]
            else:
                sk = x2skip if ti == 1 else 0
                k_ = c0//nc - sk; nu = C//nc - sk
                xs = xargs[k_*n//nu:(k_+1)*n//nu] if k_ >= 0 else []
        gs = []
        if ti == 0:
            q0 = c0//128
            gs = [(q, rp) for q in range(q0+ntl, min(NQ, q0+2*ntl)) for rp in gargs]
        ms = {}
        for jn, j in enumerate(jorder if u == 0 else range(6)):
            mine = []
            if u == 0 and jn < 2:
                allq = [(q, rp) for q in range(ntl) for rp in gargs]
                wait('w', 0)
                mine += [(gtr, a) for a in allq[jn*len(allq)//2:(jn+1)*len(allq)//2]]
            if xs and jn in xdots:
                k_ = xdots.index(jn); mx = xs[k_*len(xs)//len(xdots):(k_+1)*len(xs)//len(xdots)]
                if mx: wait('x', ti+1)
                mine += [(xtr, (ti+1,)+a) for a in mx]
            if gs and jn in gdots:
                k_ = gdots.index(jn); mg = gs[k_*len(gs)//len(gdots):(k_+1)*len(gs)//len(gdots)]
                for a in mg: wait('w', a[0])
                mine += [(gtr, a) for a in mg]
            for kd in starts.get(gdot, []): kick(*kd)
            if gdot >= odefer: flush_out(orate)
            gdot += 1
            lhs = pltpu.bitcast(tb[j, rows, :], bf16)
            if j in (0, 5):
                rw = jnp.concatenate([wi[0 if j == 0 else 2, c0//128 + q] for q in range(ntl)], axis=1)
            else:
                rw = gbuf[j-1, :, pl.ds(c0, nc)]
            loaded = []
            if mine:
                NP = ntl*2*32
                mod = {}
                for q, (fn, a) in enumerate(mine):
                    ldv = (xload if fn is xtr else gload)(*a)
                    loaded.append(ldv)
                    p = min(NP-1, ((2*q+1)*NP)//(2*len(mine)))
                    ps, r_ = p//32, p % 32
                    nt, kg = ps//2, ps % 2
                    key = ((4*kg + (r_ % 4))*8 + r_//4, nt)
                    dep = orall(ldv) & zvec
                    mod[key] = dep if key not in mod else mod[key] | dep
                rowsb = []
                for rbk in range(C//16):
                    blk = rw[8*rbk:8*rbk+8]
                    if any(k2[0] == rbk for k2 in mod):
                        blk = jnp.concatenate([(blk[:, 128*nt:128*nt+128] | mod[(rbk, nt)]) if (rbk, nt) in mod else blk[:, 128*nt:128*nt+128] for nt in range(ntl)], axis=1)
                    rowsb.append(blk)
                rw = jnp.concatenate(rowsb, axis=0)
            rhs = pltpu.bitcast(rw, bf16)
            ms[j] = jnp.dot(lhs, rhs, preferred_element_type=f32)
            for q, (fn, a) in enumerate(mine): fn(*a, loaded=loaded[q])
        for p in range(T//EG): epi(ti, c0, nc, ms, p)
        b, i = tiles[ti]
        osp = osplit if u == len(units)-1 else 1
        for q in range(ntl):
            ct = c0//128 + q
            for h in range(osp):
                rws = pl.ds(R*i + h*R//osp, R//osp)
                cp_ = pltpu.make_async_copy(obuf.at[b, ct, rws, :], o_hbm.at[b, rws, pl.ds(ct*128, 128)], osem.at[len(o_copies)])
                o_copies.append(cp_)
                if gdot > odefer + 2*len(pending_out) + 12 or u == len(units)-1:
                    flush_out(99); cp_.start()
                else:
                    pending_out.append(cp_)
    flush_out(99)
    for cp_ in o_copies: cp_.wait()
    for kd in sorted(started - waited):
        assert nunits < 32
        wait(*kd)

def _run(x, w, mean, var, g, b, T=256, NC0=128, NC1=128, XG=16, GR=16, xdepth=2, wp0=2, wp1=3, xdots='s01234', gdots='s2345',
        xsplit=4, x1units=2, wk0=2, wk1=35, xk0=23, xk1=32, xk2=41, osplit=2, nunits=99, jorder='s051234', odefer=50, orate=1, x2skip=0):
    B,S,C = x.shape
    NT = B*S//(4*T)
    dig = lambda s_: [int(ch) for ch in s_[1:]]
    hbm = pl.BlockSpec(memory_space=pl.ANY)
    return pl.pallas_call(
        functools.partial(kern, T=T, NC0=NC0, NC1=NC1, XG=XG, GR=GR, xdepth=xdepth, wp0=wp0, wp1=wp1, xdots=dig(xdots), gdots=dig(gdots), xsplit=xsplit,
                          x1units=x1units, wk=(wk0, wk1), xk=(xk0, xk1, xk2), osplit=osplit, nunits=nunits, jorder=dig(jorder), odefer=odefer, orate=orate, x2skip=x2skip),
        in_specs=[hbm]*6,
        out_specs=hbm,
        out_shape=jax.ShapeDtypeStruct((B,S,C), x.dtype),
        scratch_shapes=[
            pltpu.VMEM((B,C//128,S+32,128), bf16), pltpu.VMEM((3,C//128,C,128), bf16), pltpu.VMEM((4,C//2,C), i32),
            pltpu.VMEM((6,B*S//8,C), i32), pltpu.VMEM((B,C//128,S,128), bf16),
            pltpu.VMEM((C,), bf16), pltpu.VMEM((C,), bf16), pltpu.VMEM((C,), bf16), pltpu.VMEM((C,), bf16),
            pltpu.SemaphoreType.DMA((NT,8)), pltpu.SemaphoreType.DMA((C//128+3,)), pltpu.SemaphoreType.DMA((40,)),
            pltpu.SemaphoreType.DMA((4,)), pltpu.SemaphoreType.REGULAR,
        ],
        compiler_params=pltpu.CompilerParams(vmem_limit_bytes=100*1024*1024),
    )(x, w, mean, var, g, b)


@jax.jit
def pallas_standalone__batchnorm__prompt_kernel(x, w, mean, var, g, b):
    return _run(x, w, mean, var, g, b, )
```

```python
import functools
import jax, jax.numpy as jnp
import jax.experimental.pallas as pl
import jax.experimental.pallas.tpu as pltpu

f32 = jnp.float32; bf16 = jnp.bfloat16; i32 = jnp.int32

PA = 2.0/3.0; PB = 1.5
A2 = PA*PA; B2 = PB*PB; PP = A2 + B2
NA = 2*A2*(A2-B2); NB = 2*B2*(B2-A2)

def lo(wd): return pltpu.unpack_elementwise(wd, index=0, packed_dtype=bf16, unpacked_dtype=f32)
def hi(wd): return pltpu.unpack_elementwise(wd, index=1, packed_dtype=bf16, unpacked_dtype=f32)
def pk(a, b): return pltpu.pack_elementwise((a, b), packed_dtype=bf16)
def share(items, k, nk): return items[k*len(items)//nk:(k+1)*len(items)//nk]


def kern(x_hbm, w_hbm, mean_hbm, var_hbm, g_hbm, b_hbm, o_hbm,
         xbuf, wbuf, gbuf, tb, obuf, vb0, vb1, vb2, vb3, xsem, wsem, osem, vsem, zsem, *,
         T, GR, xdots, gdots, xsplit, xdepth, wp0, wp1, x1units, wk, xk, osplit, jorder, odefer, x2skip, x0dots):
    B, S, C = x_hbm.shape
    R = 4*T; per = S//R; NT = B*per
    NQ = C//128
    XG = EG = 16; PAD = 16
    xi = xbuf.bitcast(i32); wi = wbuf.bitcast(i32); oi = obuf.bitcast(i32)

    def x_copies(t, p=0, np_=1):
        b, i = t//per, t % per
        r0 = R*i - (16 if i > 0 else 0); r1 = R*(i+1) + (16 if i < per-1 else 0)
        if np_ > 1:
            r0 = r0 if p == 0 else R*i + p*R//np_ + 16
            r1 = r1 if p == np_-1 else R*i + (p+1)*R//np_ + 16
        return [pltpu.make_async_copy(x_hbm.at[b, pl.ds(r0, r1 - r0), pl.ds(ct*128, 128)],
                                      xbuf.at[t, ct, pl.ds(PAD + r0 - R*i, r1 - r0), :], xsem.at[t, p]) for ct in range(NQ)]
    def w_copies(q):
        return [pltpu.make_async_copy(w_hbm.at[:, :, pl.ds(q*128, 128)], wbuf.at[:, q], wsem.at[q])]
    def out_copy(t, ct, h, nsp, sem):
        b, i = t//per, t % per
        r0 = R*i + h*(R//nsp)
        if not isinstance(r0, int): r0 = pl.multiple_of(r0, 16)
        return pltpu.make_async_copy(obuf.at[t, ct, pl.ds(h*(R//nsp), R//nsp), :],
                                     o_hbm.at[b, pl.ds(r0, R//nsp), pl.ds(ct*128, 128)], osem.at[sem])
    v_copies = [pltpu.make_async_copy(r, d, vsem.at[n]) for n, (r, d) in
                enumerate(zip((mean_hbm, var_hbm, g_hbm, b_hbm), (vb0, vb1, vb2, vb3)))]
    started = set(); waited = set()
    def kick(kind, m):
        assert (kind, m) not in started
        started.add((kind, m))
        for cp in (w_copies(m) if kind == 'w' else x_copies(m)): cp.start()
    def wait(kind, m):
        assert (kind, m) in started, (kind, m)
        if (kind, m) in waited: return
        waited.add((kind, m))
        for cp in (w_copies(m) if kind == 'w' else x_copies(m)): cp.wait()

    def tile_ptr(t):
        return (t, t)
    def xload(tp, gp, cp):
        out = []
        for h in range(2):
            base = PAD//2 + 2*(gp*XG + 8*h)
            out += [xi[tp[0], cp, pl.ds(base + o, 8, stride=2), :] for o in (-1, 0, 1, 2)]
        return out
    def xtr(tp, gp, cp, loaded=None):
        ld = loaded if loaded is not None else xload(tp, gp, cp)
        ts = []
        for h in range(2):
            wa, wb, wc, wd = ld[4*h:4*h+4]
            d0, d1, d2, d3, d4, d5 = hi(wa), lo(wb), hi(wb), lo(wc), hi(wc), lo(wd)
            u1 = d4 - B2*d2; v1 = PA*(d3 - B2*d1)
            u2 = d4 - A2*d2; v2 = PB*(d3 - A2*d1)
            ts.append(((d0 + d4) - PP*d2, u1+v1, u1-v1, u2+v2, u2-v2, (d1 + d5) - PP*d3))
        for j in range(6):
            tb[tp[1], j, pl.ds(gp*XG//2, 8), pl.ds(cp*128, 128)] = pk(ts[0][j], ts[1][j])
    def gload(q, rp):
        return [wi[k, q, pl.ds(rp*GR//2, GR//2), :] for k in range(3)]
    def gtr(q, rp, loaded=None):
        wv = loaded if loaded is not None else gload(q, rp)
        res = []
        for h in (lo, hi):
            w0, w1, w2 = h(wv[0]), h(wv[1]), h(wv[2])
            sa = w0*(1.0/NA) + w2*(A2/NA); da = w1*(PA/NA)
            sb = w0*(1.0/NB) + w2*(B2/NB); db = w1*(PB/NB)
            res.append((sa+da, sa-da, sb+db, sb-db))
        for j in range(4):
            gbuf[j, pl.ds(rp*GR//2, GR//2), pl.ds(q*128, 128)] = pk(res[0][j], res[1][j])

    zvec = jnp.full((8, 128), pl.semaphore_read(zsem), i32)
    def do_dot(j, t, ct, mine):
        lhs = pltpu.bitcast(tb[t, j], bf16)
        rw = wi[0 if j == 0 else 2, ct] if j in (0, 5) else gbuf[j-1, :, pl.ds(ct*128, 128)]
        loaded = []
        if mine:
            mod = {}
            for q, (fn, a) in enumerate(mine):
                ldv = (xload if fn is xtr else gload)(*a)
                loaded.append(ldv)
                p = min(63, ((2*q+1)*64)//(2*len(mine)))
                key = (4*(p//32) + (p % 4))*8 + (p % 32)//4
                dep = functools.reduce(lambda u, v: u | v, ldv) & zvec
                mod[key] = dep if key not in mod else mod[key] | dep
            rw = jnp.concatenate([(rw[8*r:8*r+8] | mod[r]) if r in mod else rw[8*r:8*r+8] for r in range(C//16)], axis=0)
        m = jnp.dot(lhs, pltpu.bitcast(rw, bf16), preferred_element_type=f32)
        for q, (fn, a) in enumerate(mine): fn(*a, loaded=loaded[q])
        return m

    for p in range(min(xdepth, xsplit)):
        for cp in x_copies(0, p, xsplit): cp.start()
    for cp in v_copies: cp.start()
    zpad = jnp.zeros((PAD//2, 128), i32)
    for t in range(NT):
        for ct in range(NQ):
            if t % per == 0: xi[t, ct, pl.ds(0, PAD//2), :] = zpad
            if t % per == per-1: xi[t, ct, pl.ds((PAD + R)//2, PAD//2), :] = zpad
    xargs = [(gp, cp) for gp in range(T//XG) for cp in range(NQ)]
    gargs = list(range(C//GR))
    for p in range(xsplit):
        for cp in x_copies(0, p, xsplit): cp.wait()
        if p+xdepth < xsplit:
            for cp in x_copies(0, p+xdepth, xsplit): cp.start()
        if p == min(xsplit-1, wp0): kick('w', 0)
        if p == min(xsplit-1, wp1): kick('w', 1)
        for a in share(xargs, p, xsplit): xtr(tile_ptr(0), *a)
    for cp in v_copies: cp.wait()
    mean, var, g, bb = [r[...].astype(f32).reshape(1, C) for r in (vb0, vb1, vb2, vb3)]
    scale = 0.5 * g * jax.lax.rsqrt(var + 1e-5)
    shift = 0.5 * bb - mean*scale

    def epi(t, ct, ms, part):
        sl = slice(part*EG, (part+1)*EG)
        m0, m1, m2, m3, m4, m5 = [ms[j][sl] for j in range(6)]
        sa = m1 + m2; da = m1 - m2; sb = m3 + m4; db = m3 - m4
        y0 = m0 + sa + sb
        y1 = PA*da + PB*db
        y2 = A2*sa + B2*sb
        y3 = (PA*A2)*da + (PB*B2)*db + m5
        sc = scale[:, ct*128:ct*128+128]; sh = shift[:, ct*128:ct*128+128]
        def act(y):
            h = y*sc + sh
            return h + h*jnp.tanh(h)
        w01 = pk(act(y0), act(y1)); w23 = pk(act(y2), act(y3))
        ev = jax.lax.broadcasted_iota(i32, (8, 128), 0) % 2 == 0
        wbase = 2*part*EG
        for h in range(2):
            a_ = w01[8*h:8*h+8]; b_ = w23[8*h:8*h+8]
            oi[t, ct, pl.ds(wbase + 8*h, 8), :] = jnp.where(ev, a_, pltpu.roll(b_, 1, 0))
            oi[t, ct, pl.ds(wbase + 16 + 8*h, 8), :] = jnp.where(ev, pltpu.roll(a_, 7, 0), b_)

    starts = {}
    for q in range(2, NQ): starts.setdefault(wk[0] + ((q-2)*wk[1])//10, []).append(('w', q))
    for t in range(1, NT): starts.setdefault(xk[t-1], []).append(('x', t))
    gdot = 0
    for u in range(NQ):
        us = list(range(NQ - x1units, NQ))
        xs = share(xargs, us.index(u), len(us)) if u in us else []
        gs = [(u+1, rp) for rp in gargs] if u+1 < NQ else []
        ms = {}
        for jn, j in enumerate(jorder if u == 0 else range(6)):
            mine = []
            if u == 0 and jn < 2:
                wait('w', 0)
                mine += [(gtr, (0, rp)) for rp in share(gargs, jn, 2)]
            if xs and jn in x0dots:
                wait('x', 1)
                mine += [(xtr, (tile_ptr(1),)+a) for a in share(xs, x0dots.index(jn), len(x0dots))]
            if gs and jn in gdots:
                wait('w', u+1)
                mine += [(gtr, a) for a in share(gs, gdots.index(jn), len(gdots))]
            for kd in starts.get(gdot, []): kick(*kd)
            gdot += 1
            ms[j] = do_dot(j, 0, u, mine)
        for p in range(T//EG): epi(0, u, ms, p)
    assert per == 2 and NT == 4
    assert started - waited == {('x', t) for t in range(2, NT)}

    def tile_body(ti, carry):
        nxt = jnp.minimum(ti + 1, NT - 1)
        for t in range(2, NT):
            @pl.when(ti + 1 == t)
            def _():
                for cp in x_copies(t): cp.wait()
        @pl.when(ti == odefer)
        def _():
            for u in range(NQ): out_copy(0, u, 0, 1, u).start()
        tpn = (nxt, ti + 1)
        for u in range(NQ):
            xs = share(xargs, u - x2skip, NQ - x2skip) if u >= x2skip else []
            ms = {}
            for j in range(6):
                mine = [(xtr, (tpn,)+a) for a in share(xs, xdots.index(j), len(xdots))] if j in xdots else []
                ms[j] = do_dot(j, ti, u, mine)
            for p in range(T//EG): epi(ti, u, ms, p)
            for h in range(osplit):
                out_copy(ti, u, h, osplit, NQ + ((ti-1)*NQ + u)*osplit + h).start()
        return carry
    jax.lax.fori_loop(1, NT, tile_body, 0)

    for u in range(NQ): out_copy(0, u, 0, 1, u).wait()
    for t in range(1, NT):
        for u in range(NQ):
            for h in range(osplit):
                out_copy(t, u, h, osplit, NQ + ((t-1)*NQ + u)*osplit + h).wait()


def _run(x, w, mean, var, g, b, T=256, GR=16, xdots='s01234', x0dots='s01234', gdots='s2345', xsplit=4, xdepth=2, wp0=2, wp1=3,
        x1units=2, wk0=2, wk1=35, xk0=23, xk1=32, xk2=41, osplit=1, jorder='s051234', odefer=2, x2skip=0):
    B, S, C = x.shape
    NT = B*S//(4*T); NQ = C//128
    dig = lambda s: [int(ch) for ch in s[1:]]
    hbm = pl.BlockSpec(memory_space=pl.ANY)
    return pl.pallas_call(
        functools.partial(kern, T=T, GR=GR, xdots=dig(xdots), x0dots=dig(x0dots), gdots=dig(gdots), xsplit=xsplit, xdepth=xdepth, wp0=wp0, wp1=wp1,
                          x1units=x1units, wk=(wk0, wk1), xk=(xk0, xk1, xk2), osplit=osplit, jorder=dig(jorder), odefer=odefer, x2skip=x2skip),
        in_specs=[hbm]*6,
        out_specs=hbm,
        out_shape=jax.ShapeDtypeStruct((B, S, C), x.dtype),
        scratch_shapes=[
            pltpu.VMEM((NT, NQ, 4*T+32, 128), bf16), pltpu.VMEM((3, NQ, C, 128), bf16), pltpu.VMEM((4, C//2, C), i32),
            pltpu.VMEM((NT+1, 6, T//2, C), i32), pltpu.VMEM((NT, NQ, 4*T, 128), bf16),
            pltpu.VMEM((C,), bf16), pltpu.VMEM((C,), bf16), pltpu.VMEM((C,), bf16), pltpu.VMEM((C,), bf16),
            pltpu.SemaphoreType.DMA((NT, 8)), pltpu.SemaphoreType.DMA((NQ,)), pltpu.SemaphoreType.DMA((NQ*(1 + (NT-1)*osplit),)),
            pltpu.SemaphoreType.DMA((4,)), pltpu.SemaphoreType.REGULAR,
        ],
        compiler_params=pltpu.CompilerParams(vmem_limit_bytes=100*1024*1024),
    )(x, w, mean, var, g, b)


@jax.jit
def pallas_standalone__batchnorm__prompt_kernel(x, w, mean, var, g, b):
    return _run(x, w, mean, var, g, b, )
```

```python
import functools
import jax, jax.numpy as jnp
import jax.experimental.pallas as pl
import jax.experimental.pallas.tpu as pltpu

f32 = jnp.float32; bf16 = jnp.bfloat16; i32 = jnp.int32

PA = 2.0/3.0; PB = 1.5
A2 = PA*PA; B2 = PB*PB; PP = A2 + B2
NA = 2*A2*(A2-B2); NB = 2*B2*(B2-A2)

def lo(wd): return pltpu.unpack_elementwise(wd, index=0, packed_dtype=bf16, unpacked_dtype=f32)
def hi(wd): return pltpu.unpack_elementwise(wd, index=1, packed_dtype=bf16, unpacked_dtype=f32)
def pk(a, b): return pltpu.pack_elementwise((a, b), packed_dtype=bf16)
def share(items, k, nk): return items[k*len(items)//nk:(k+1)*len(items)//nk]


def kern(x_hbm, w_hbm, mean_hbm, var_hbm, g_hbm, b_hbm, o_hbm,
         xbuf, wbuf, gbuf, tb, obuf, vb0, vb1, vb2, vb3, xsem, wsem, osem, vsem, zsem, *,
         T, GR, xdots, gdots, xsplit, xdepth, wp0, wp1, x1units, wk, xk, osplit, jorder, odefer, x2skip, x0dots, pfirst, g0dots, wgroup, gpro, nstatic):
    B, S, C = x_hbm.shape
    R = 4*T; per = S//R; NT = B*per
    NQ = C//128
    XG = EG = 16; PAD = 16
    xi = xbuf.bitcast(i32); wi = wbuf.bitcast(i32); oi = obuf.bitcast(i32)

    def x_copies(t, p=0, np_=1):
        b, i = t//per, t % per
        r0 = R*i - (16 if i > 0 else 0); r1 = R*(i+1) + (16 if i < per-1 else 0)
        if np_ > 1:
            r0 = r0 if p == 0 else R*i + p*R//np_ + 16
            r1 = r1 if p == np_-1 else R*i + (p+1)*R//np_ + 16
        return [pltpu.make_async_copy(x_hbm.at[b, pl.ds(r0, r1 - r0), pl.ds(ct*128, 128)],
                                      xbuf.at[t, ct, pl.ds(PAD + r0 - R*i, r1 - r0), :], xsem.at[t, p]) for ct in range(NQ)]
    def w_copies(q):
        return [pltpu.make_async_copy(w_hbm.at[:, :, pl.ds(q*128, 128)], wbuf.at[:, q], wsem.at[q])]
    def out_copy(t, ct, h, nsp, sem):
        b, i = t//per, t % per
        r0 = R*i + h*(R//nsp)
        if not isinstance(r0, int): r0 = pl.multiple_of(r0, 16)
        return pltpu.make_async_copy(obuf.at[t, ct, pl.ds(h*(R//nsp), R//nsp), :],
                                     o_hbm.at[b, pl.ds(r0, R//nsp), pl.ds(ct*128, 128)], osem.at[sem])
    v_copies = [pltpu.make_async_copy(r, d, vsem.at[n]) for n, (r, d) in
                enumerate(zip((mean_hbm, var_hbm, g_hbm, b_hbm), (vb0, vb1, vb2, vb3)))]
    started = set(); waited = set()
    def kick(kind, m):
        assert (kind, m) not in started
        started.add((kind, m))
        for cp in (w_copies(m) if kind == 'w' else x_copies(m)): cp.start()
    def wait(kind, m):
        assert (kind, m) in started, (kind, m)
        if (kind, m) in waited: return
        waited.add((kind, m))
        for cp in (w_copies(m) if kind == 'w' else x_copies(m)): cp.wait()

    def tile_ptr(t):
        return (t, t)
    def xload(tp, gp, cp):
        out = []
        for h in range(2):
            base = PAD//2 + 2*(gp*XG + 8*h)
            out += [xi[tp[0], cp, pl.ds(base + o, 8, stride=2), :] for o in (-1, 0, 1, 2)]
        return out
    def xtr(tp, gp, cp, loaded=None):
        ld = loaded if loaded is not None else xload(tp, gp, cp)
        ts = []
        for h in range(2):
            wa, wb, wc, wd = ld[4*h:4*h+4]
            d0, d1, d2, d3, d4, d5 = hi(wa), lo(wb), hi(wb), lo(wc), hi(wc), lo(wd)
            u1 = d4 - B2*d2; v1 = PA*(d3 - B2*d1)
            u2 = d4 - A2*d2; v2 = PB*(d3 - A2*d1)
            ts.append(((d0 + d4) - PP*d2, u1+v1, u1-v1, u2+v2, u2-v2, (d1 + d5) - PP*d3))
        for j in range(6):
            tb[tp[1], j, pl.ds(gp*XG//2, 8), pl.ds(cp*128, 128)] = pk(ts[0][j], ts[1][j])
    def gload(q, rp):
        return [wi[k, q, pl.ds(rp*GR//2, GR//2), :] for k in range(3)]
    def gtr(q, rp, loaded=None):
        wv = loaded if loaded is not None else gload(q, rp)
        res = []
        for h in (lo, hi):
            w0, w1, w2 = h(wv[0]), h(wv[1]), h(wv[2])
            sa = w0*(1.0/NA) + w2*(A2/NA); da = w1*(PA/NA)
            sb = w0*(1.0/NB) + w2*(B2/NB); db = w1*(PB/NB)
            res.append((sa+da, sa-da, sb+db, sb-db))
        for j in range(4):
            gbuf[j, pl.ds(rp*GR//2, GR//2), pl.ds(q*128, 128)] = pk(res[0][j], res[1][j])

    zvec = jnp.full((8, 128), pl.semaphore_read(zsem), i32)
    def do_dot(j, t, ct, mine, pmin=0):
        lhs = pltpu.bitcast(tb[t, j], bf16)
        rw = wi[0 if j == 0 else 2, ct] if j in (0, 5) else gbuf[j-1, :, pl.ds(ct*128, 128)]
        loaded = []
        if mine:
            mod = {}
            for q, (fn, a) in enumerate(mine):
                ldv = (xload if fn is xtr else gload)(*a)
                loaded.append(ldv)
                p = min(63, pmin + ((2*q+1)*(64 - pmin))//(2*len(mine)))
                key = (4*(p//32) + (p % 4))*8 + (p % 32)//4
                dep = functools.reduce(lambda u, v: u | v, ldv) & zvec
                mod[key] = dep if key not in mod else mod[key] | dep
            rw = jnp.concatenate([(rw[8*r:8*r+8] | mod[r]) if r in mod else rw[8*r:8*r+8] for r in range(C//16)], axis=0)
        m = jnp.dot(lhs, pltpu.bitcast(rw, bf16), preferred_element_type=f32)
        for q, (fn, a) in enumerate(mine): fn(*a, loaded=loaded[q])
        return m

    if gpro >= 0: kick('w', 0)
    for p in range(min(xdepth, xsplit)):
        for cp in x_copies(0, p, xsplit): cp.start()
    for cp in v_copies: cp.start()
    zpad = jnp.zeros((PAD//2, 128), i32)
    for t in range(NT):
        for ct in range(NQ):
            if t % per == 0: xi[t, ct, pl.ds(0, PAD//2), :] = zpad
            if t % per == per-1: xi[t, ct, pl.ds((PAD + R)//2, PAD//2), :] = zpad
    xargs = [(gp, cp) for gp in range(T//XG) for cp in range(NQ)]
    gargs = list(range(C//GR))
    for p in range(xsplit):
        for cp in x_copies(0, p, xsplit): cp.wait()
        if p+xdepth < xsplit:
            for cp in x_copies(0, p+xdepth, xsplit): cp.start()
        if gpro < 0 and p == min(xsplit-1, wp0): kick('w', 0)
        if p == min(xsplit-1, wp1): kick('w', 1)
        for a in share(xargs, p, xsplit): xtr(tile_ptr(0), *a)
        if p == gpro:
            wait('w', 0)
            for rp in gargs: gtr(0, rp)
    for cp in v_copies: cp.wait()
    mean, var, g, bb = [r[...].astype(f32).reshape(1, C) for r in (vb0, vb1, vb2, vb3)]
    scale = 0.5 * g * jax.lax.rsqrt(var + 1e-5)
    shift = 0.5 * bb - mean*scale

    def epi(t, ct, ms, part):
        sl = slice(part*EG, (part+1)*EG)
        m0, m1, m2, m3, m4, m5 = [ms[j][sl] for j in range(6)]
        sa = m1 + m2; da = m1 - m2; sb = m3 + m4; db = m3 - m4
        y0 = m0 + sa + sb
        y1 = PA*da + PB*db
        y2 = A2*sa + B2*sb
        y3 = (PA*A2)*da + (PB*B2)*db + m5
        sc = scale[:, ct*128:ct*128+128]; sh = shift[:, ct*128:ct*128+128]
        def act(y):
            h = y*sc + sh
            return h + h*jnp.tanh(h)
        w01 = pk(act(y0), act(y1)); w23 = pk(act(y2), act(y3))
        ev = jax.lax.broadcasted_iota(i32, (8, 128), 0) % 2 == 0
        wbase = 2*part*EG
        for h in range(2):
            a_ = w01[8*h:8*h+8]; b_ = w23[8*h:8*h+8]
            oi[t, ct, pl.ds(wbase + 8*h, 8), :] = jnp.where(ev, a_, pltpu.roll(b_, 1, 0))
            oi[t, ct, pl.ds(wbase + 16 + 8*h, 8), :] = jnp.where(ev, pltpu.roll(a_, 7, 0), b_)

    starts = {}
    for q in range(2, NQ): starts.setdefault(wk[0] + ((q-2)*wk[1])//10, []).append(('w', q))
    for t in range(1, NT): starts.setdefault(xk[t-1], []).append(('x', t))
    gdot = 0
    for u in range(NQ):
        us = list(range(NQ - x1units, NQ))
        xs = share(xargs, us.index(u), len(us)) if u in us else []
        gs = [(u+1, rp) for rp in gargs] if u+1 < NQ else []
        ms = {}
        for jn, j in enumerate(jorder if u == 0 else range(6)):
            mine = []; nw = len(waited)
            if u == 0 and jn < 2 and gpro < 0:
                wait('w', 0)
                mine += [(gtr, (0, rp)) for rp in share(gargs, jn, 2)]
            if xs and jn in x0dots:
                wait('x', 1)
                mine += [(xtr, (tile_ptr(1),)+a) for a in share(xs, x0dots.index(jn), len(x0dots))]
            gd = g0dots if u == 0 else gdots
            if gs and jn in gd:
                for q in wgroup[u+1]: wait('w', q)
                mine += [(gtr, a) for a in share(gs, gd.index(jn), len(gd))]
            for kd in starts.get(gdot, []): kick(*kd)
            gdot += 1
            ms[j] = do_dot(j, 0, u, mine, pfirst if len(waited) > nw else 0)
        for p in range(T//EG): epi(0, u, ms, p)
    assert per == 2 and NT == 4
    assert started - waited == {('x', t) for t in range(2, NT)}

    def tile_body(ti, carry):
        if isinstance(ti, int):
            nxt = min(ti + 1, NT - 1)
            if ti + 1 < NT:
                for cp in x_copies(ti + 1): cp.wait()
        else:
            nxt = jnp.minimum(ti + 1, NT - 1)
            for t in range(nstatic + 1, NT):
                @pl.when(ti + 1 == t)
                def _():
                    for cp in x_copies(t): cp.wait()
        if isinstance(ti, int):
            if ti == odefer:
                for u in range(NQ): out_copy(0, u, 0, 1, u).start()
        elif odefer >= nstatic:
            @pl.when(ti == odefer)
            def _():
                for u in range(NQ): out_copy(0, u, 0, 1, u).start()
        tpn = (nxt, ti + 1)
        for u in range(NQ):
            xs = share(xargs, u - x2skip, NQ - x2skip) if u >= x2skip else []
            ms = {}
            for j in range(6):
                mine = [(xtr, (tpn,)+a) for a in share(xs, xdots.index(j), len(xdots))] if j in xdots else []
                ms[j] = do_dot(j, ti, u, mine)
            for p in range(T//EG): epi(ti, u, ms, p)
            for h in range(osplit):
                out_copy(ti, u, h, osplit, NQ + ((ti-1)*NQ + u)*osplit + h).start()
        return carry
    for t_ in range(1, nstatic): tile_body(t_, 0)
    if nstatic < NT: jax.lax.fori_loop(nstatic, NT, tile_body, 0)

    for u in range(NQ): out_copy(0, u, 0, 1, u).wait()
    for t in range(1, NT):
        for u in range(NQ):
            for h in range(osplit):
                out_copy(t, u, h, osplit, NQ + ((t-1)*NQ + u)*osplit + h).wait()


def _run(x, w, mean, var, g, b, T=256, GR=16, xdots='s01234', x0dots='s01234', gdots='s0134', xsplit=4, xdepth=2, wp0=2, wp1=3,
        x1units=2, wk0=1, wk1=30, xk0=20, xk1=30, xk2=40, osplit=1, jorder='s051234', odefer=2, x2skip=0, pfirst=36, g0dots='s234', wg='s12346', gpro=-1, nstatic=1):
    B, S, C = x.shape
    NT = B*S//(4*T); NQ = C//128
    dig = lambda s: [int(ch) for ch in s[1:]]
    gs_ = dig(wg)
    wgroup = {q: (list(range(q, ([e for e in gs_ if e > q] + [NQ])[0])) if q in gs_ else []) for q in range(1, NQ)}
    hbm = pl.BlockSpec(memory_space=pl.ANY)
    return pl.pallas_call(
        functools.partial(kern, T=T, GR=GR, xdots=dig(xdots), x0dots=dig(x0dots), gdots=dig(gdots), xsplit=xsplit, xdepth=xdepth, wp0=wp0, wp1=wp1,
                          x1units=x1units, wk=(wk0, wk1), xk=(xk0, xk1, xk2), osplit=osplit, jorder=dig(jorder), odefer=odefer, x2skip=x2skip, pfirst=pfirst, g0dots=dig(g0dots), wgroup=wgroup, gpro=gpro, nstatic=nstatic),
        in_specs=[hbm]*6,
        out_specs=hbm,
        out_shape=jax.ShapeDtypeStruct((B, S, C), x.dtype),
        scratch_shapes=[
            pltpu.VMEM((NT, NQ, 4*T+32, 128), bf16), pltpu.VMEM((3, NQ, C, 128), bf16), pltpu.VMEM((4, C//2, C), i32),
            pltpu.VMEM((NT+1, 6, T//2, C), i32), pltpu.VMEM((NT, NQ, 4*T, 128), bf16),
            pltpu.VMEM((C,), bf16), pltpu.VMEM((C,), bf16), pltpu.VMEM((C,), bf16), pltpu.VMEM((C,), bf16),
            pltpu.SemaphoreType.DMA((NT, 8)), pltpu.SemaphoreType.DMA((NQ,)), pltpu.SemaphoreType.DMA((NQ*(1 + (NT-1)*osplit),)),
            pltpu.SemaphoreType.DMA((4,)), pltpu.SemaphoreType.REGULAR,
        ],
        compiler_params=pltpu.CompilerParams(vmem_limit_bytes=100*1024*1024),
    )(x, w, mean, var, g, b)


@jax.jit
def pallas_standalone__batchnorm__prompt_kernel(x, w, mean, var, g, b):
    return _run(x, w, mean, var, g, b, )
```

```python
import functools
import jax, jax.numpy as jnp
import jax.experimental.pallas as pl
import jax.experimental.pallas.tpu as pltpu

f32 = jnp.float32; bf16 = jnp.bfloat16; i32 = jnp.int32

PA = 2.0/3.0; PB = 1.5
A2 = PA*PA; B2 = PB*PB; PP = A2 + B2
NA = 2*A2*(A2-B2); NB = 2*B2*(B2-A2)

def lo(wd): return pltpu.unpack_elementwise(wd, index=0, packed_dtype=bf16, unpacked_dtype=f32)
def hi(wd): return pltpu.unpack_elementwise(wd, index=1, packed_dtype=bf16, unpacked_dtype=f32)
def pk(a, b): return pltpu.pack_elementwise((a, b), packed_dtype=bf16)
def share(items, k, nk): return items[k*len(items)//nk:(k+1)*len(items)//nk]


def kern(x_hbm, w_hbm, mean_hbm, var_hbm, g_hbm, b_hbm, o_hbm,
         xbuf, wbuf, gbuf, tb, obuf, pbuf, vb0, vb1, vb2, vb3, xsem, wsem, osem, vsem, zsem, *,
         T, GR, xdots, gdots, x1units, wk, xk, osplit, odefer, x2skip, x0dots, pfirst, g0dots, wgroup, nstatic, xbdots, hks):
    B, S, C = x_hbm.shape
    R = 4*T; per = S//R; NT = B*per
    NQ = C//128
    XG = EG = 16; PAD = 16
    xi = xbuf.bitcast(i32); wi = wbuf.bitcast(i32); oi = obuf.bitcast(i32)

    def x_copies(t, p=0, np_=1):
        b, i = t//per, t % per
        r0 = R*i - (16 if i > 0 else 0); r1 = R*(i+1) + (16 if i < per-1 else 0)
        if np_ > 1:
            r0 = r0 if p == 0 else R*i + p*R//np_ + 16
            r1 = r1 if p == np_-1 else R*i + (p+1)*R//np_ + 16
        return [pltpu.make_async_copy(x_hbm.at[b, pl.ds(r0, r1 - r0), pl.ds(ct*128, 128)],
                                      xbuf.at[t, ct, pl.ds(PAD + r0 - R*i, r1 - r0), :], xsem.at[t, p]) for ct in range(NQ)]
    def w_copies(q):
        return [pltpu.make_async_copy(w_hbm.at[:, :, pl.ds(q*128, 128)], wbuf.at[:, q], wsem.at[q])]
    def x0_copies(kh, p):
        r0 = 0 if p == 0 else R//2 + 16; r1 = R//2 + 16 if p == 0 else R + 16
        return [pltpu.make_async_copy(x_hbm.at[0, pl.ds(r0, r1 - r0), pl.ds(ct*128, 128)],
                                      xbuf.at[0, ct, pl.ds(PAD + r0, r1 - r0), :], xsem.at[0, 2*kh + p]) for ct in range(kh*NQ//2, (kh+1)*NQ//2)]
    def wh_copies(q, kh):
        rows = pl.ds(kh*C//2, C//2)
        return [pltpu.make_async_copy(w_hbm.at[:, rows, pl.ds(q*128, 128)], wbuf.at[:, q, rows, :], wsem.at[NQ + 2*q + kh])]
    def out_copy(t, ct, h, nsp, sem):
        b, i = t//per, t % per
        r0 = R*i + h*(R//nsp)
        if not isinstance(r0, int): r0 = pl.multiple_of(r0, 16)
        return pltpu.make_async_copy(obuf.at[t, ct, pl.ds(h*(R//nsp), R//nsp), :],
                                     o_hbm.at[b, pl.ds(r0, R//nsp), pl.ds(ct*128, 128)], osem.at[sem])
    v_copies = [pltpu.make_async_copy(r, d, vsem.at[n]) for n, (r, d) in
                enumerate(zip((mean_hbm, var_hbm, g_hbm, b_hbm), (vb0, vb1, vb2, vb3)))]
    COPIES = {'w': w_copies, 'x': x_copies, 'x0': x0_copies, 'wh': wh_copies}
    started = set(); waited = set()
    def kick(kind, *m):
        assert (kind, m) not in started
        started.add((kind, m))
        for cp in COPIES[kind](*m): cp.start()
    def wait(kind, *m):
        assert (kind, m) in started, (kind, m)
        if (kind, m) in waited: return
        waited.add((kind, m))
        for cp in COPIES[kind](*m): cp.wait()

    def tile_ptr(t):
        return (t, t)
    def xload(tp, gp, cp):
        out = []
        for h in range(2):
            base = PAD//2 + 2*(gp*XG + 8*h)
            out += [xi[tp[0], cp, pl.ds(base + o, 8, stride=2), :] for o in (-1, 0, 1, 2)]
        return out
    def xtr(tp, gp, cp, loaded=None):
        ld = loaded if loaded is not None else xload(tp, gp, cp)
        ts = []
        for h in range(2):
            wa, wb, wc, wd = ld[4*h:4*h+4]
            d0, d1, d2, d3, d4, d5 = hi(wa), lo(wb), hi(wb), lo(wc), hi(wc), lo(wd)
            u1 = d4 - B2*d2; v1 = PA*(d3 - B2*d1)
            u2 = d4 - A2*d2; v2 = PB*(d3 - A2*d1)
            ts.append(((d0 + d4) - PP*d2, u1+v1, u1-v1, u2+v2, u2-v2, (d1 + d5) - PP*d3))
        for j in range(6):
            tb[tp[1], j, pl.ds(gp*XG//2, 8), pl.ds(cp*128, 128)] = pk(ts[0][j], ts[1][j])
    def gload(q, rp):
        return [wi[k, q, pl.ds(rp*GR//2, GR//2), :] for k in range(3)]
    def gtr(q, rp, loaded=None):
        wv = loaded if loaded is not None else gload(q, rp)
        res = []
        for h in (lo, hi):
            w0, w1, w2 = h(wv[0]), h(wv[1]), h(wv[2])
            sa = w0*(1.0/NA) + w2*(A2/NA); da = w1*(PA/NA)
            sb = w0*(1.0/NB) + w2*(B2/NB); db = w1*(PB/NB)
            res.append((sa+da, sa-da, sb+db, sb-db))
        for j in range(4):
            gbuf[j, pl.ds(rp*GR//2, GR//2), pl.ds(q*128, 128)] = pk(res[0][j], res[1][j])

    zero = pl.semaphore_read(zsem)
    zvec = jnp.full((8, 128), zero, i32)
    def do_dot(j, t, ct, mine, pmin=0, kh=None):
        k0, kn = (0, C) if kh is None else (kh*C//2, C//2)
        lhs = pltpu.bitcast(tb[t, j, :, pl.ds(k0, kn)], bf16)
        wrows = pl.ds(k0//2, kn//2)
        rw = wi[0 if j == 0 else 2, ct, wrows, :] if j in (0, 5) else gbuf[j-1, wrows, pl.ds(ct*128, 128)]
        NP = kn//16
        loaded = []
        if mine:
            mod = {}
            for q, (fn, a) in enumerate(mine):
                ldv = (xload if fn is xtr else gload)(*a)
                loaded.append(ldv)
                pm = min(pmin, NP//2)
                p = min(NP-1, pm + ((2*q+1)*(NP - pm))//(2*len(mine)))
                key = (4*(p//32) + (p % 4))*8 + (p % 32)//4
                dep = functools.reduce(lambda u, v: u | v, ldv) & zvec
                mod[key] = dep if key not in mod else mod[key] | dep
            rw = jnp.concatenate([(rw[8*r:8*r+8] | mod[r]) if r in mod else rw[8*r:8*r+8] for r in range(NP)], axis=0)
        m = jnp.dot(lhs, pltpu.bitcast(rw, bf16), preferred_element_type=f32)
        for q, (fn, a) in enumerate(mine): fn(*a, loaded=loaded[q])
        return m

    kick('x0', 0, 0); kick('x0', 0, 1); kick('wh', 0, 0)
    for cp in v_copies: cp.start()
    zpad = jnp.zeros((PAD//2, 128), i32)
    for t in range(NT):
        for ct in range(NQ):
            if t % per == 0: xi[t, ct, pl.ds(0, PAD//2), :] = zpad
            if t % per == per-1: xi[t, ct, pl.ds((PAD + R)//2, PAD//2), :] = zpad
    xargs = [(gp, cp) for gp in range(T//XG) for cp in range(NQ)]
    gargs = list(range(C//GR))
    x0args = lambda kh, p: [(gp, cp) for gp, cp in xargs if cp//(NQ//2) == kh and gp//(T//XG//2) == p]
    wait('x0', 0, 0); kick('wh', 1, 0)
    for a in x0args(0, 0): xtr(tile_ptr(0), *a)
    wait('x0', 0, 1); kick('x0', 1, 0); kick('x0', 1, 1)
    for a in x0args(0, 1): xtr(tile_ptr(0), *a)
    for cp in v_copies: cp.wait()
    mean, var, g, bb = [r[...].astype(f32).reshape(1, C) for r in (vb0, vb1, vb2, vb3)]
    scale = 0.5 * g * jax.lax.rsqrt(var + 1e-5)
    shift = 0.5 * bb - mean*scale

    def epi(t, ct, ms, part):
        sl = slice(part*EG, (part+1)*EG)
        m0, m1, m2, m3, m4, m5 = [ms[j][sl] for j in range(6)]
        sa = m1 + m2; da = m1 - m2; sb = m3 + m4; db = m3 - m4
        y0 = m0 + sa + sb
        y1 = PA*da + PB*db
        y2 = A2*sa + B2*sb
        y3 = (PA*A2)*da + (PB*B2)*db + m5
        sc = scale[:, ct*128:ct*128+128]; sh = shift[:, ct*128:ct*128+128]
        def act(y):
            h = y*sc + sh
            return h + h*jnp.tanh(h)
        w01 = pk(act(y0), act(y1)); w23 = pk(act(y2), act(y3))
        ev = jax.lax.broadcasted_iota(i32, (8, 128), 0) % 2 == 0
        wbase = 2*part*EG
        for h in range(2):
            a_ = w01[8*h:8*h+8]; b_ = w23[8*h:8*h+8]
            oi[t, ct, pl.ds(wbase + 8*h, 8), :] = jnp.where(ev, a_, pltpu.roll(b_, 1, 0))
            oi[t, ct, pl.ds(wbase + 16 + 8*h, 8), :] = jnp.where(ev, pltpu.roll(a_, 7, 0), b_)

    hk = {}
    for pos, item in zip(hks, (('wh', 0, 1), ('wh', 1, 1), ('w', 2), ('w', 3), ('w', 4), ('w', 5))):
        hk.setdefault((pos//6, pos % 6), []).append(item)
    def half_step(s_, q, kh):
        gh = share(gargs, kh, 2)
        ms = {}
        for jn, j in enumerate((0, 5, 1, 2, 3, 4) if q == 0 else range(6)):
            mine = []; nw = len(waited)
            if q == 0 and jn < 2:
                wait('wh', 0, kh); mine += [(gtr, (0, rp)) for rp in share(gh, jn, 2)]
            if q == 0 and 2 <= jn < 5:
                wait('wh', 1, kh); mine += [(gtr, (1, rp)) for rp in share(gh, jn - 2, 3)]
            if s_ == 1 and jn in xbdots:
                wait('x0', 1, 0); wait('x0', 1, 1)
                mine += [(xtr, (tile_ptr(0),)+a) for a in share(x0args(1, 0) + x0args(1, 1), xbdots.index(jn), len(xbdots))]
            if s_ == 3 and jn in g0dots:
                wait('w', 2); mine += [(gtr, (2, rp)) for rp in share(gargs, g0dots.index(jn), len(g0dots))]
            for item in hk.get((s_, jn), []): kick(*item)
            m = do_dot(j, 0, q, mine, pfirst if len(waited) > nw else 0, kh)
            if kh == 0: pbuf[q, j] = m
            else: ms[j] = pbuf[q, j] + m
        if kh == 1:
            for p in range(T//EG): epi(0, q, ms, p)
    @pl.when(zero == 0)
    def _():
        half_step(0, 0, 0)
        half_step(1, 1, 0)
    half_step(2, 0, 1)
    half_step(3, 1, 1)
    starts = {wk[0]: [('w', 6)], wk[1]: [('w', 7)]}
    for t in range(1, NT): starts.setdefault(xk[t-1], []).append(('x', t))
    gdot = 0
    for u in range(2, NQ):
        us = list(range(NQ - x1units, NQ))
        xs = share(xargs, us.index(u), len(us)) if u in us else []
        gs = [(u+1, rp) for rp in gargs] if u+1 < NQ else []
        ms = {}
        for j in range(6):
            mine = []; nw = len(waited)
            if xs and j in x0dots:
                wait('x', 1)
                mine += [(xtr, (tile_ptr(1),)+a) for a in share(xs, x0dots.index(j), len(x0dots))]
            if gs and j in gdots:
                for q in wgroup[u+1]: wait('w', q)
                mine += [(gtr, a) for a in share(gs, gdots.index(j), len(gdots))]
            for kd in starts.get(gdot, []): kick(*kd)
            gdot += 1
            ms[j] = do_dot(j, 0, u, mine, pfirst if len(waited) > nw else 0)
        for p in range(T//EG): epi(0, u, ms, p)
    assert per == 2 and NT == 4
    assert started - waited == {('x', (t,)) for t in range(2, NT)}, started - waited

    def tile_body(ti, carry):
        if isinstance(ti, int):
            nxt = min(ti + 1, NT - 1)
            if ti + 1 < NT:
                for cp in x_copies(ti + 1): cp.wait()
        else:
            nxt = jnp.minimum(ti + 1, NT - 1)
            for t in range(nstatic + 1, NT):
                @pl.when(ti + 1 == t)
                def _():
                    for cp in x_copies(t): cp.wait()
        if isinstance(ti, int):
            if ti == odefer:
                for u in range(NQ): out_copy(0, u, 0, 1, u).start()
        elif odefer >= nstatic:
            @pl.when(ti == odefer)
            def _():
                for u in range(NQ): out_copy(0, u, 0, 1, u).start()
        tpn = (nxt, ti + 1)
        for u in range(NQ):
            xs = share(xargs, u - x2skip, NQ - x2skip) if u >= x2skip else []
            ms = {}
            for j in range(6):
                mine = [(xtr, (tpn,)+a) for a in share(xs, xdots.index(j), len(xdots))] if j in xdots else []
                ms[j] = do_dot(j, ti, u, mine)
            for p in range(T//EG): epi(ti, u, ms, p)
            for h in range(osplit):
                out_copy(ti, u, h, osplit, NQ + ((ti-1)*NQ + u)*osplit + h).start()
        return carry
    for t_ in range(1, nstatic): tile_body(t_, 0)
    if nstatic < NT: jax.lax.fori_loop(nstatic, NT, tile_body, 0)

    for u in range(NQ): out_copy(0, u, 0, 1, u).wait()
    for t in range(1, NT):
        for u in range(NQ):
            for h in range(osplit):
                out_copy(t, u, h, osplit, NQ + ((t-1)*NQ + u)*osplit + h).wait()


def _run(x, w, mean, var, g, b, T=256, GR=16, xdots='s01234', x0dots='s01234', gdots='s0134', x1units=2,
        wk0=1, wk1=4, xk0=8, xk1=18, xk2=28, osplit=1, odefer=2, x2skip=0, pfirst=36, g0dots='s2345', wg='s346', nstatic=1, xbdots='s45', hks='h04.07.10.13.16.19'):
    B, S, C = x.shape
    NT = B*S//(4*T); NQ = C//128
    dig = lambda s: [int(ch) for ch in s[1:]]
    gs_ = dig(wg)
    wgroup = {q: (list(range(q, ([e for e in gs_ if e > q] + [NQ])[0])) if q in gs_ else []) for q in range(1, NQ)}
    hbm = pl.BlockSpec(memory_space=pl.ANY)
    return pl.pallas_call(
        functools.partial(kern, T=T, GR=GR, xdots=dig(xdots), x0dots=dig(x0dots), gdots=dig(gdots), x1units=x1units, wk=(wk0, wk1),
                          xk=(xk0, xk1, xk2), osplit=osplit, odefer=odefer, x2skip=x2skip, pfirst=pfirst, g0dots=dig(g0dots),
                          wgroup=wgroup, nstatic=nstatic, xbdots=dig(xbdots), hks=[int(v) for v in hks[1:].split('.')]),
        in_specs=[hbm]*6,
        out_specs=hbm,
        out_shape=jax.ShapeDtypeStruct((B, S, C), x.dtype),
        scratch_shapes=[
            pltpu.VMEM((NT, NQ, 4*T+32, 128), bf16), pltpu.VMEM((3, NQ, C, 128), bf16), pltpu.VMEM((4, C//2, C), i32),
            pltpu.VMEM((NT+1, 6, T//2, C), i32), pltpu.VMEM((NT, NQ, 4*T, 128), bf16), pltpu.VMEM((2, 6, T, 128), f32),
            pltpu.VMEM((C,), bf16), pltpu.VMEM((C,), bf16), pltpu.VMEM((C,), bf16), pltpu.VMEM((C,), bf16),
            pltpu.SemaphoreType.DMA((NT, 8)), pltpu.SemaphoreType.DMA((NQ + 4,)), pltpu.SemaphoreType.DMA((NQ*(1 + (NT-1)*osplit),)),
            pltpu.SemaphoreType.DMA((4,)), pltpu.SemaphoreType.REGULAR,
        ],
        compiler_params=pltpu.CompilerParams(vmem_limit_bytes=100*1024*1024),
    )(x, w, mean, var, g, b)


@jax.jit
def pallas_standalone__batchnorm__prompt_kernel(x, w, mean, var, g, b):
    return _run(x, w, mean, var, g, b, )
```

```python
import functools

import jax
import jax.numpy as jnp
import jax.experimental.pallas as pl
import jax.experimental.pallas.tpu as pltpu

f32, bf16, i32 = jnp.float32, jnp.bfloat16, jnp.int32

PA, PB = 2.0 / 3.0, 1.5
A2, B2 = PA * PA, PB * PB
PP = A2 + B2
NA, NB = 2 * A2 * (A2 - B2), 2 * B2 * (B2 - A2)

T = 256
XG = 16
GR = 16
PAD = 16
XDOTS = (0, 1, 2, 3, 4)
GDOTS = (0, 1, 3, 4)
W_GROUPS = (3, 4, 6)
HALF_KICKS = (4, 7, 10, 13, 16, 19)
W_KICKS = {1: 6, 4: 7}
X_KICKS = {8: 1, 18: 2, 28: 3}
OUT0_TILE = 2


def lo(wd): return pltpu.unpack_elementwise(wd, index=0, packed_dtype=bf16, unpacked_dtype=f32)
def hi(wd): return pltpu.unpack_elementwise(wd, index=1, packed_dtype=bf16, unpacked_dtype=f32)
def pk(a, b): return pltpu.pack_elementwise((a, b), packed_dtype=bf16)
def share(items, k, nk): return items[k * len(items) // nk:(k + 1) * len(items) // nk]


def _kernel(x_hbm, w_hbm, mean_hbm, var_hbm, g_hbm, b_hbm, o_hbm,
            xbuf, wbuf, gbuf, tb, obuf, pbuf, vb0, vb1, vb2, vb3, xsem, wsem, osem, vsem, zsem):
    B, S, C = x_hbm.shape
    R = 4 * T; per = S // R; NT = B * per
    NQ = C // 128
    xi, wi, oi = xbuf.bitcast(i32), wbuf.bitcast(i32), obuf.bitcast(i32)

    def x_copies(t):
        b, i = t // per, t % per
        r0 = R * i - (PAD if i > 0 else 0); r1 = R * (i + 1) + (PAD if i < per - 1 else 0)
        return [pltpu.make_async_copy(x_hbm.at[b, pl.ds(r0, r1 - r0), pl.ds(ct * 128, 128)],
                                      xbuf.at[t, ct, pl.ds(PAD + r0 - R * i, r1 - r0), :], xsem.at[t, 0])
                for ct in range(NQ)]
    def x0_copies(kh, p):
        r0 = 0 if p == 0 else R // 2 + PAD
        r1 = R // 2 + PAD if p == 0 else R + (PAD if per > 1 else 0)
        return [pltpu.make_async_copy(x_hbm.at[0, pl.ds(r0, r1 - r0), pl.ds(ct * 128, 128)],
                                      xbuf.at[0, ct, pl.ds(PAD + r0, r1 - r0), :], xsem.at[0, 2 * kh + p])
                for ct in range(kh * NQ // 2, (kh + 1) * NQ // 2)]
    def w_copies(q):
        return [pltpu.make_async_copy(w_hbm.at[:, :, pl.ds(q * 128, 128)], wbuf.at[:, q], wsem.at[q])]
    def wh_copies(q, kh):
        rows = pl.ds(kh * C // 2, C // 2)
        return [pltpu.make_async_copy(w_hbm.at[:, rows, pl.ds(q * 128, 128)], wbuf.at[:, q, rows, :],
                                      wsem.at[NQ + 2 * q + kh])]
    def out_copy(t, ct):
        r0 = R * (t % per)
        if not isinstance(r0, int): r0 = pl.multiple_of(r0, R)
        return pltpu.make_async_copy(obuf.at[t, ct], o_hbm.at[t // per, pl.ds(r0, R), pl.ds(ct * 128, 128)],
                                     osem.at[t * NQ + ct])
    v_copies = [pltpu.make_async_copy(r, d, vsem.at[n]) for n, (r, d) in
                enumerate(zip((mean_hbm, var_hbm, g_hbm, b_hbm), (vb0, vb1, vb2, vb3)))]
    copies = {'w': w_copies, 'x': x_copies, 'x0': x0_copies, 'wh': wh_copies}
    started, waited = set(), set()
    def kick(kind, *m):
        assert (kind, m) not in started
        started.add((kind, m))
        for cp in copies[kind](*m): cp.start()
    def wait(kind, *m):
        assert (kind, m) in started, (kind, m)
        if (kind, m) not in waited:
            waited.add((kind, m))
            for cp in copies[kind](*m): cp.wait()

    def xload(src, dst, gp, cp):
        out = []
        for h in range(2):
            base = PAD // 2 + 2 * (gp * XG + 8 * h)
            out += [xi[src, cp, pl.ds(base + o, 8, stride=2), :] for o in (-1, 0, 1, 2)]
        return out
    def xtr(src, dst, gp, cp, loaded=None):
        ld = loaded if loaded is not None else xload(src, dst, gp, cp)
        ts = []
        for h in range(2):
            wa, wb, wc, wd = ld[4 * h:4 * h + 4]
            d0, d1, d2, d3, d4, d5 = hi(wa), lo(wb), hi(wb), lo(wc), hi(wc), lo(wd)
            u1 = d4 - B2 * d2; v1 = PA * (d3 - B2 * d1)
            u2 = d4 - A2 * d2; v2 = PB * (d3 - A2 * d1)
            ts.append(((d0 + d4) - PP * d2, u1 + v1, u1 - v1, u2 + v2, u2 - v2, (d1 + d5) - PP * d3))
        for j in range(6):
            tb[dst, j, pl.ds(gp * XG // 2, 8), pl.ds(cp * 128, 128)] = pk(ts[0][j], ts[1][j])
    def gload(q, rp):
        return [wi[k, q, pl.ds(rp * GR // 2, GR // 2), :] for k in range(3)]
    def gtr(q, rp, loaded=None):
        wv = loaded if loaded is not None else gload(q, rp)
        res = []
        for h in (lo, hi):
            w0, w1, w2 = h(wv[0]), h(wv[1]), h(wv[2])
            sa = w0 * (1.0 / NA) + w2 * (A2 / NA); da = w1 * (PA / NA)
            sb = w0 * (1.0 / NB) + w2 * (B2 / NB); db = w1 * (PB / NB)
            res.append((sa + da, sa - da, sb + db, sb - db))
        for j in range(4):
            gbuf[j, pl.ds(rp * GR // 2, GR // 2), pl.ds(q * 128, 128)] = pk(res[0][j], res[1][j])
    loader = {xtr: xload, gtr: gload}

    zero = pl.semaphore_read(zsem)
    zvec = jnp.full((8, 128), zero, i32)

    def product(j, t, ct, tasks, late=False, kh=None):
        k0, kn = (0, C) if kh is None else (kh * C // 2, C // 2)
        lhs = pltpu.bitcast(tb[t, j, :, pl.ds(k0, kn)], bf16)
        wrows = pl.ds(k0 // 2, kn // 2)
        rw = wi[0 if j == 0 else 2, ct, wrows, :] if j in (0, 5) else gbuf[j - 1, wrows, pl.ds(ct * 128, 128)]
        npos = kn // 16
        p0 = min(36, npos // 2) if late else 0
        loaded, mod = [], {}
        for n, (fn, a) in enumerate(tasks):
            ld = loader[fn](*a)
            loaded.append(ld)
            p = min(npos - 1, p0 + ((2 * n + 1) * (npos - p0)) // (2 * len(tasks)))
            reg = (4 * (p // 32) + p % 4) * 8 + (p % 32) // 4
            dep = functools.reduce(lambda u, v: u | v, ld) & zvec
            mod[reg] = dep if reg not in mod else mod[reg] | dep
        if mod:
            rw = jnp.concatenate([(rw[8 * r:8 * r + 8] | mod[r]) if r in mod else rw[8 * r:8 * r + 8]
                                  for r in range(npos)], axis=0)
        m = jnp.dot(lhs, pltpu.bitcast(rw, bf16), preferred_element_type=f32)
        for (fn, a), ld in zip(tasks, loaded): fn(*a, loaded=ld)
        return m

    kick('x0', 0, 0); kick('x0', 0, 1); kick('wh', 0, 0)
    for cp in v_copies: cp.start()
    zpad = jnp.zeros((PAD // 2, 128), i32)
    for t in range(NT):
        for ct in range(NQ):
            if t % per == 0: xi[t, ct, pl.ds(0, PAD // 2), :] = zpad
            if t % per == per - 1: xi[t, ct, pl.ds((PAD + R) // 2, PAD // 2), :] = zpad
    xargs = [(gp, cp) for gp in range(T // XG) for cp in range(NQ)]
    gargs = list(range(C // GR))
    def x0args(kh, p):
        return [(gp, cp) for gp, cp in xargs if cp // (NQ // 2) == kh and gp // (T // XG // 2) == p]
    wait('x0', 0, 0); kick('wh', 1, 0)
    for a in x0args(0, 0): xtr(0, 0, *a)
    wait('x0', 0, 1); kick('x0', 1, 0); kick('x0', 1, 1)
    for a in x0args(0, 1): xtr(0, 0, *a)
    for cp in v_copies: cp.wait()
    mean, var, gamma, beta = [r[...].astype(f32).reshape(1, C) for r in (vb0, vb1, vb2, vb3)]
    scale = 0.5 * gamma * jax.lax.rsqrt(var + 1e-5)
    shift = 0.5 * beta - mean * scale

    def epilogue(t, ct, ms):
        sc = scale[:, ct * 128:ct * 128 + 128]; sh = shift[:, ct * 128:ct * 128 + 128]
        def act(y):
            h = y * sc + sh
            return h + h * jnp.tanh(h)
        even = jax.lax.broadcasted_iota(i32, (8, 128), 0) % 2 == 0
        for p in range(T // XG):
            m0, m1, m2, m3, m4, m5 = [ms[j][p * XG:(p + 1) * XG] for j in range(6)]
            sa = m1 + m2; da = m1 - m2; sb = m3 + m4; db = m3 - m4
            y0 = m0 + sa + sb
            y1 = PA * da + PB * db
            y2 = A2 * sa + B2 * sb
            y3 = (PA * A2) * da + (PB * B2) * db + m5
            w01 = pk(act(y0), act(y1)); w23 = pk(act(y2), act(y3))
            for h in range(2):
                a = w01[8 * h:8 * h + 8]; b_ = w23[8 * h:8 * h + 8]
                oi[t, ct, pl.ds(2 * p * XG + 8 * h, 8), :] = jnp.where(even, a, pltpu.roll(b_, 1, 0))
                oi[t, ct, pl.ds(2 * p * XG + 16 + 8 * h, 8), :] = jnp.where(even, pltpu.roll(a, 7, 0), b_)

    early = {}
    for pos, item in zip(HALF_KICKS, (('wh', 0, 1), ('wh', 1, 1), ('w', 2), ('w', 3), ('w', 4), ('w', 5))):
        early.setdefault(pos, []).append(item)
    def half_unit(step, q, kh):
        gh = share(gargs, kh, 2)
        ms = {}
        for n, j in enumerate((0, 5, 1, 2, 3, 4) if q == 0 else range(6)):
            tasks = []; nw = len(waited)
            if q == 0 and n < 2:
                wait('wh', 0, kh); tasks += [(gtr, (0, rp)) for rp in share(gh, n, 2)]
            if q == 0 and 2 <= n < 5:
                wait('wh', 1, kh); tasks += [(gtr, (1, rp)) for rp in share(gh, n - 2, 3)]
            if step == 1 and n >= 4:
                wait('x0', 1, 0); wait('x0', 1, 1)
                tasks += [(xtr, (0, 0) + a) for a in share(x0args(1, 0) + x0args(1, 1), n - 4, 2)]
            if step == 3 and n >= 2:
                wait('w', 2); tasks += [(gtr, (2, rp)) for rp in share(gargs, n - 2, 4)]
            for item in early.get(6 * step + n, []): kick(*item)
            m = product(j, 0, q, tasks, len(waited) > nw, kh)
            if kh == 0: pbuf[q, j] = m
            else: ms[j] = pbuf[q, j] + m
        if kh == 1: epilogue(0, q, ms)

    @pl.when(zero == 0)
    def _():
        half_unit(0, 0, 0)
        half_unit(1, 1, 0)
    half_unit(2, 0, 1)
    half_unit(3, 1, 1)

    slot = 0
    for u in range(2, NQ):
        xs = share(xargs, u - (NQ - 2), 2) if u >= NQ - 2 else []
        gs = [(u + 1, rp) for rp in gargs] if u + 1 < NQ else []
        ms = {}
        for j in range(6):
            tasks = []; nw = len(waited)
            if xs and j in XDOTS:
                wait('x', 1)
                tasks += [(xtr, (1, 1) + a) for a in share(xs, XDOTS.index(j), len(XDOTS))]
            if gs and j in GDOTS:
                if u + 1 in W_GROUPS:
                    for q in range(u + 1, min([e for e in W_GROUPS if e > u + 1] + [NQ])): wait('w', q)
                tasks += [(gtr, a) for a in share(gs, GDOTS.index(j), len(GDOTS))]
            if slot in W_KICKS: kick('w', W_KICKS[slot])
            if slot in X_KICKS: kick('x', X_KICKS[slot])
            slot += 1
            ms[j] = product(j, 0, u, tasks, len(waited) > nw)
        epilogue(0, u, ms)
    assert started - waited == {('x', (t,)) for t in range(2, NT)}

    def tile_body(ti, carry):
        nxt = jnp.minimum(ti + 1, NT - 1)
        for t in range(2, NT):
            @pl.when(ti + 1 == t)
            def _():
                for cp in x_copies(t): cp.wait()
        @pl.when(ti == OUT0_TILE)
        def _():
            for u in range(NQ): out_copy(0, u).start()
        for u in range(NQ):
            xs = share(xargs, u, NQ)
            ms = {}
            for j in range(6):
                tasks = [(xtr, (nxt, ti + 1) + a) for a in share(xs, XDOTS.index(j), len(XDOTS))] if j in XDOTS else []
                ms[j] = product(j, ti, u, tasks)
            epilogue(ti, u, ms)
            out_copy(ti, u).start()
        return carry
    jax.lax.fori_loop(1, NT, tile_body, 0)

    for t in range(NT):
        for u in range(NQ): out_copy(t, u).wait()


@jax.jit
def pallas_standalone__batchnorm__prompt_kernel(x, w, mean, var, g, b):
    B, S, C = x.shape
    NT, NQ = B * S // (4 * T), C // 128
    assert w.shape == (3, C, C) and S % (4 * T) == 0 and NT == 4 and S // (4 * T) == 2 and NQ == 8
    hbm = pl.BlockSpec(memory_space=pl.ANY)
    return pl.pallas_call(
        _kernel,
        in_specs=[hbm] * 6,
        out_specs=hbm,
        out_shape=jax.ShapeDtypeStruct((B, S, C), x.dtype),
        scratch_shapes=[
            pltpu.VMEM((NT, NQ, 4 * T + 2 * PAD, 128), bf16),
            pltpu.VMEM((3, NQ, C, 128), bf16),
            pltpu.VMEM((4, C // 2, C), i32),
            pltpu.VMEM((NT + 1, 6, T // 2, C), i32),
            pltpu.VMEM((NT, NQ, 4 * T, 128), bf16),
            pltpu.VMEM((2, 6, T, 128), f32),
            pltpu.VMEM((C,), bf16), pltpu.VMEM((C,), bf16), pltpu.VMEM((C,), bf16), pltpu.VMEM((C,), bf16),
            pltpu.SemaphoreType.DMA((NT, 4)), pltpu.SemaphoreType.DMA((NQ + 4,)),
            pltpu.SemaphoreType.DMA((NT * NQ,)), pltpu.SemaphoreType.DMA((4,)),
            pltpu.SemaphoreType.REGULAR,
        ],
        compiler_params=pltpu.CompilerParams(vmem_limit_bytes=100 * 1024 * 1024),
    )(x, w, mean, var, g, b)
```
